```python
import os as _os
_os.environ.setdefault("JAX_PLATFORMS", "cpu")
import jax
import jax.numpy as jnp

def _softmax(x, axis=-1):
    return jax.nn.softmax(x, axis=axis)
def _gelu(x):
    return jax.nn.gelu(x, approximate=True)
def _silu(x):
    return jax.nn.silu(x)
def _sigmoid(x):
    return jax.nn.sigmoid(x)
def _layernorm(x, axis=-1, eps=1e-5):
    m = jnp.mean(x, axis=axis, keepdims=True)
    v = jnp.var(x, axis=axis, keepdims=True)
    return (x - m) / jnp.sqrt(v + eps)
def _scatter_add(tgt, idx, src, axis=0):
    return tgt.at[idx].add(src)
def _segment_sum(src, seg, n):
    return jax.ops.segment_sum(src, seg, n)
class _Rng:
    def __init__(self, key):
        self._k = key
    def _next(self):
        self._k, sub = jax.random.split(self._k)
        return sub
    def normal(self, shape):
        return jax.random.normal(self._next(), shape, dtype=jnp.bfloat16)
    def randint(self, lo, hi, shape):
        return jax.random.randint(self._next(), shape, lo, hi, dtype=jnp.int32)
    def uniform(self, shape, lo=0.0, hi=1.0):
        return jax.random.uniform(self._next(), shape, jnp.bfloat16, lo, hi)
    def permutation(self, n):
        return jax.random.permutation(self._next(), n)


kernel_name = 'interleave_layers__mha_block__mixer_s_mlp__prompt'

def setup_inputs():
    _rng = _Rng(jax.random.key(int.from_bytes(__import__("os").urandom(4), "little")))
    _w = (lambda a: (lambda t: t.astype(jnp.bfloat16) if jnp.issubdtype(t.dtype, jnp.floating) else t)(jnp.asarray(a)))
    def _A_setup():
        B, S, D, H = 1, 2048, 448, 16
        return {
            "x": _w((lambda *s: _rng.normal(s) * 0.05)(B, S, D)),
            "wqkv": _w((lambda *s: _rng.normal(s) * 0.05)(D, 3 * D)),
            "wo": _w((lambda *s: _rng.normal(s) * 0.05)(D, D)),
        }
    _A_in = _A_setup()

    def _B_setup():
        B, S, D, F = 1, 2048, 448, 1792
        return {
            "x":  _w((lambda *s: _rng.normal(s) * 0.05)(B, S, D)),
            "w1": _w((lambda *s: _rng.normal(s) * 0.8)(D, D) * (D ** -0.5)),
            "w2": _w((lambda *s: _rng.normal(s) * 0.8)(D, D) * (D ** -0.5)),
            "w3": _w((lambda *s: _rng.normal(s) * 0.8)(D, F) * (D ** -0.5)),
            "w4": _w((lambda *s: _rng.normal(s) * 0.8)(F, D) * (F ** -0.5)),
        }
    _B_in = _B_setup()

    return {
        "A_x": _A_in["x"],
        "A_wqkv": _A_in["wqkv"],
        "A_wo": _A_in["wo"],
        "B_x": _B_in["x"],
        "B_w1": _B_in["w1"],
        "B_w2": _B_in["w2"],
        "B_w3": _B_in["w3"],
        "B_w4": _B_in["w4"],
    }

def reference(A_x, A_wqkv, A_wo, B_x, B_w1, B_w2, B_w3, B_w4):
    def _A_ref(x, wqkv, wo):
        B, S, D = x.shape
        H = 16
        Dh = D // H
        qkv = (lambda x, *d: x.transpose(*d))((x @ wqkv).reshape(B, S, 3, H, Dh), 2, 0, 3, 1, 4)
        q, k, v = qkv[0], qkv[1], qkv[2]
        scores = jnp.einsum("bhqd,bhkd->bhqk", q, k) * (Dh ** -0.5)
        p = _softmax(scores, axis=-1)
        o = jnp.einsum("bhqk,bhkd->bhqd", p, v)
        return (lambda x, *d: x.transpose(*d))(o, 0, 2, 1, 3).reshape(B, S, D) @ wo

    def _B_ref(x, w1, w2, w3, w4):
        B, S, D = x.shape
        h = _gelu(_layernorm(x, axis=-1) @ w1)
        c = D // 4
        g0 = jnp.pad(h[:, :, 0*c:1*c], ((0, 0), (1, 0), (0, 0)))[:, :S, :]
        g1 = jnp.pad(h[:, :, 1*c:2*c], ((0, 0), (0, 1), (0, 0)))[:, 1:, :]
        g2 = jnp.pad(h[:, :, 2*c:3*c], ((0, 0), (2, 0), (0, 0)))[:, :S, :]
        g3 = jnp.pad(h[:, :, 3*c:   ], ((0, 0), (0, 2), (0, 0)))[:, 2:, :]
        hs = jnp.concatenate([g0, g1, g2, g3], axis=-1) @ w2
        x1 = x + hs
        h2 = _gelu(_layernorm(x1, axis=-1) @ w3) @ w4
        return x1 + h2

    x = A_x
    x = x + _A_ref(_layernorm(x, axis=-1), A_wqkv, A_wo)
    x = x + _B_ref(_layernorm(x, axis=-1), B_w1, B_w2, B_w3, B_w4)
    x = x + _A_ref(_layernorm(x, axis=-1), A_wqkv, A_wo)
    x = x + _B_ref(_layernorm(x, axis=-1), B_w1, B_w2, B_w3, B_w4)
    return x
```

```python
import math

import jax
import jax.numpy as jnp
from jax import lax
from jax.experimental import pallas as pl
from jax.experimental.pallas import tpu as pltpu

S = 2048
D = 448
H = 16
DH = D // H
F = 1792
TB = 512
NTB = S // TB
KC = 128
NC = S // KC
HG = 4
GW = HG * DH
C4 = D // 4
EPS = 1e-5
QSCALE = (DH ** -0.5) * math.log2(math.e)

f32 = jnp.float32
bf16 = jnp.bfloat16


def _ln(x):
    t = x.shape[1]
    s = jnp.sum(jnp.sum(x.reshape(D // 8, 8, t), axis=0), axis=0, keepdims=True)
    xc = x - s * (1.0 / D)
    v = jnp.sum(jnp.sum((xc * xc).reshape(D // 8, 8, t), axis=0), axis=0, keepdims=True)
    return xc * lax.rsqrt(v * (1.0 / D) + EPS)


def _gelu(x):
    c = math.sqrt(2.0 / math.pi)
    u = x * (c + (c * 0.044715) * (x * x))
    hx = 0.5 * x
    return hx + hx * jnp.tanh(u)


def _dot(a, b):
    return jnp.dot(a, b, preferred_element_type=f32)


def _kernel(x_hbm, wqkv_hbm, wo_hbm, w1_hbm, w2_hbm, w3_hbm, w4_hbm, o_hbm,
            x_in, wqkv_in, wo_in, w1_in, w2_in, w3_in, w4_in,
            wqkv_t, wo_t, w1_t, w2_t, w3_t, w4_t,
            xt, yt, qt, kk, vt, ot, sbuf, hbuf, obuf, sems):
    srcs = (wqkv_hbm, x_hbm, wo_hbm, w1_hbm, w2_hbm, w3_hbm, w4_hbm)
    dsts = (wqkv_in, x_in, wo_in, w1_in, w2_in, w3_in, w4_in)
    copies = [pltpu.make_async_copy(s, d, sems.at[i]) for i, (s, d) in enumerate(zip(srcs, dsts))]
    for c in copies:
        c.start()

    hbuf[:, 0:128] = jnp.zeros((D, 128), bf16)
    hbuf[:, 128 + S:256 + S] = jnp.zeros((D, 128), bf16)
    sbuf[...] = jnp.zeros(sbuf.shape, f32)

    copies[0].wait()
    wqkv_t[...] = wqkv_in[...].T
    copies[1].wait()
    xt[...] = x_in[...].astype(f32)
    for c, src, dst in ((copies[2], wo_in, wo_t), (copies[3], w1_in, w1_t), (copies[4], w2_in, w2_t),
                        (copies[5], w3_in, w3_t)):
        c.wait()
        dst[...] = src[...].T
    copies[6].wait()
    w4_t[...] = w4_in[...]

    def qkv_block(b, _):
        t0 = pl.multiple_of(b * TB, TB)
        y = _ln(xt[:, pl.ds(t0, TB)]).astype(bf16)
        q = _dot(wqkv_t[0:D, :], y)
        qt[:, pl.ds(t0, TB)] = (q * QSCALE).astype(bf16)
        k = _dot(wqkv_t[D:2 * D, :], y)
        for g in range(H // HG):
            kg = jnp.concatenate([k[g * GW:(g + 1) * GW, :], jnp.zeros((128 - GW, TB), f32)], axis=0)
            kk[g, pl.ds(t0, TB), :] = kg.T.astype(bf16)
        v = _dot(wqkv_t[2 * D:3 * D, :], y)
        row = lax.broadcasted_iota(jnp.int32, (8, TB), 0)
        for h in range(H):
            r0 = (DH * h) // 8 * 8
            if h % 2 == 0:
                last = jnp.where(row < 4, v[r0 + 24:r0 + 32, :], 1.0)
                vh = jnp.concatenate([v[r0:r0 + 24, :], last], axis=0)
            else:
                first = jnp.where(row >= 4, v[r0:r0 + 8, :], 1.0)
                vh = jnp.concatenate([first, v[r0 + 8:r0 + 32, :]], axis=0)
            vt[h, :, pl.ds(t0, TB)] = vh.astype(bf16)
        return 0

    def attn_step(i, mprev, odd):
        ic = jnp.minimum(i, H * NTB - 1)
        ip = jnp.maximum(i - 1, 0)
        h = (ic // (2 * NTB)) * 2 + ic % 2
        qb = (ic // 2) % NTB
        hp = (ip // (2 * NTB)) * 2 + ip % 2
        qbp = (ip // 2) % NTB
        g = h // HG
        q0 = pl.multiple_of(qb * TB, TB)
        g0 = pl.multiple_of(g * GW, 16)
        qg = qt[pl.ds(g0, GW), pl.ds(q0, TB)]
        row = lax.broadcasted_iota(jnp.int32, (GW, TB), 0)
        lo = (h % HG) * DH
        qm = jnp.where((row >= lo) & (row < lo + DH), qg, jnp.zeros_like(qg))
        qm = jnp.concatenate([qm, jnp.zeros((128 - GW, TB), bf16)], axis=0)
        mx = None
        acc = None
        for c in range(NC):
            st = _dot(kk[g, c * KC:(c + 1) * KC, :], qm)
            sp = sbuf[c * KC:(c + 1) * KC, :]
            t = jnp.max(st.reshape(KC // 8, 8, TB), axis=0)
            mx = t if mx is None else jnp.maximum(mx, t)
            p = jnp.exp2(sp - mprev).astype(bf16)
            sbuf[c * KC:(c + 1) * KC, :] = st
            d = _dot(vt[hp, :, c * KC:(c + 1) * KC], p)
            acc = d if acc is None else acc + d
        l = acc[28:29, :] if odd else acc[0:1, :]
        return jnp.max(mx, axis=0, keepdims=True), acc * (1.0 / l), hp, qbp

    def attn_pair(j, carry):
        m, oe = carry
        m, oo, hp, qbp = attn_step(2 * j, m, False)
        row = lax.broadcasted_iota(jnp.int32, (8, TB), 0)
        mid = jnp.where(row < 4, oe[24:32, :], oo[0:8, :])
        o = jnp.concatenate([oe[0:24, :], mid, oo[8:32, :]], axis=0)
        r0 = pl.multiple_of((hp // 2) * (2 * DH), 8)
        ot[pl.ds(r0, 2 * DH), pl.ds(pl.multiple_of(qbp * TB, TB), TB)] = o
        m, oe, _, _ = attn_step(2 * j + 1, m, True)
        return m, oe

    def mix1_block(b, _):
        t0 = pl.multiple_of(b * TB, TB)
        x = xt[:, pl.ds(t0, TB)] + _dot(wo_t[...], ot[:, pl.ds(t0, TB)].astype(bf16))
        y = _ln(x)
        xt[:, pl.ds(t0, TB)] = x
        yt[:, pl.ds(t0, TB)] = y
        h = _gelu(_dot(w1_t[...], _ln(y).astype(bf16)))
        hbuf[:, pl.ds(pl.multiple_of(t0 + 128, 128), TB)] = h.astype(bf16)
        return 0

    def mix2_block(b, _):
        t0 = pl.multiple_of(b * TB, TB)
        gs = []
        for j, sh in enumerate((1, -1, 2, -2)):
            w = hbuf[j * C4:(j + 1) * C4, pl.ds(t0, TB + 256)]
            gs.append(w[:, 128 - sh:128 - sh + TB])
        g = jnp.concatenate(gs, axis=0)
        x1 = yt[:, pl.ds(t0, TB)] + _dot(w2_t[...], g)
        u = _ln(x1).astype(bf16)
        t = _gelu(_dot(w3_t[...], u)).astype(bf16)
        h2 = _dot(w4_t[...], t)
        xt[:, pl.ds(t0, TB)] = xt[:, pl.ds(t0, TB)] + (x1 + h2)
        return 0

    def layer(_, carry):
        lax.fori_loop(0, NTB, qkv_block, 0)
        lax.fori_loop(0, H * NTB // 2 + 1, attn_pair,
                      (jnp.zeros((1, TB), f32), jnp.zeros((32, TB), f32)))
        lax.fori_loop(0, NTB, mix1_block, 0)
        lax.fori_loop(0, NTB, mix2_block, 0)
        return carry

    lax.fori_loop(0, 2, layer, 0)

    outs = []
    for b in range(NTB):
        obuf[:, b * TB:(b + 1) * TB] = xt[:, b * TB:(b + 1) * TB].astype(bf16)
        cp = pltpu.make_async_copy(obuf.at[:, pl.ds(b * TB, TB)], o_hbm.at[:, pl.ds(b * TB, TB)], sems.at[7 + b])
        cp.start()
        outs.append(cp)
    for cp in outs:
        cp.wait()


@jax.jit
def pallas_interleave_layers__mha_block__mixer_s_mlp__prompt_kernel(
        A_x, A_wqkv, A_wo, B_x, B_w1, B_w2, B_w3, B_w4):
    del B_x
    vmem = pltpu.VMEM
    any_spec = pl.BlockSpec(memory_space=pltpu.HBM)
    out = pl.pallas_call(
        _kernel,
        out_shape=jax.ShapeDtypeStruct((D, S), A_x.dtype),
        in_specs=[any_spec] * 7,
        out_specs=any_spec,
        scratch_shapes=[
            vmem((D, S), bf16), vmem((D, 3 * D), bf16), vmem((D, D), bf16), vmem((D, D), bf16),
            vmem((D, D), bf16), vmem((D, F), bf16), vmem((D, F), bf16),
            vmem((3 * D, D), bf16), vmem((D, D), bf16), vmem((D, D), bf16), vmem((D, D), bf16),
            vmem((F, D), bf16), vmem((D, F), bf16),
            vmem((D, S), f32), vmem((D, S), f32), vmem((D, S), bf16), vmem((H // HG, S, 128), bf16),
            vmem((H, 32, S), bf16), vmem((D, S), f32), vmem((S, TB), f32), vmem((D, S + 256), bf16),
            vmem((D, S), bf16),
            pltpu.SemaphoreType.DMA((7 + NTB,)),
        ],
        compiler_params=pltpu.CompilerParams(vmem_limit_bytes=110 * 2 ** 20),
    )(A_x.reshape(S, D).T, A_wqkv, A_wo, B_w1, B_w2, B_w3, B_w4.T)
    return out.T.reshape(1, S, D)
```

```python
import math

import jax
import jax.numpy as jnp
from jax import lax
from jax.experimental import pallas as pl
from jax.experimental.pallas import tpu as pltpu

S = 2048
D = 448
H = 16
DH = D // H
F = 1792
DHF = D // 2
DHP = 256
FHF = F // 2
DQ = D // 4
NT = 256
TB = 2 * NT
NB = S // TB
NU = F // 256
QB = 512
NQ = S // QB
KC = 128
NC = S // KC
HG = 4
GW = HG * DH
C4 = D // 4
NV = 192
SCORE_BOUND = 60.0
VALUE_BOUND = 2.0 ** 40
QCH = (112,)
KCH = (112,)
VCH = (112,)
UCH = (32, 32)
EPS = 1e-5
QSCALE = (DH ** -0.5) * math.log2(math.e)

f32 = jnp.float32
bf16 = jnp.bfloat16
u32 = jnp.uint32


def _pack(x):
    return pltpu.bitcast(x.astype(bf16), u32)


def _unpack(x):
    return pltpu.bitcast(x, bf16)


def _rowsum8(x):
    return jnp.sum(x.reshape(x.shape[0] // 8, 8, x.shape[1]), axis=0)


def _colsum(x8):
    return jnp.sum(x8, axis=0, keepdims=True)


def _gelu2(x):
    c = math.sqrt(2.0 / math.pi)
    return x + x * jnp.tanh(x * (c + (c * 0.044715) * (x * x)))


def _dot(a, b):
    return jnp.dot(a, b, preferred_element_type=f32)


def _split(blocks):
    n = len(blocks) // 2
    return ([r[:n] for r in blocks[:n]], [r[n:] for r in blocks[:n]],
            [r[:n] for r in blocks[n:]], [r[n:] for r in blocks[n:]])


def _add(x, y):
    return [[a + b for a, b in zip(r, s)] for r, s in zip(x, y)]


def _sub(x, y):
    return [[a - b for a, b in zip(r, s)] for r, s in zip(x, y)]


def _lhs_terms(blocks):
    if len(blocks) == 1:
        return [blocks[0][0]]
    a11, a12, a21, a22 = _split(blocks)
    terms = (_add(a11, a22), _add(a21, a22), a11, a22, _add(a11, a12), _sub(a21, a11), _sub(a12, a22))
    return [t for x in terms for t in _lhs_terms(x)]


def _rhs_terms(blocks):
    if len(blocks) == 1:
        return [blocks[0][0]]
    b11, b12, b21, b22 = _split(blocks)
    terms = (_add(b11, b22), b11, _sub(b12, b22), _sub(b21, b11), b22, _add(b11, b12), _add(b21, b22))
    return [t for x in terms for t in _rhs_terms(x)]


def _strassen(n, prod, issued, base=0):
    if n == 1:
        issued.append(prod(base))
        return [[issued[-1]]]
    stride = 7 ** (n.bit_length() - 2)

    def m(i):
        return _strassen(n // 2, prod, issued, base + i * stride)

    m1 = m(0)
    m2 = m(1)
    c22 = _sub(m1, m2)
    m4 = m(3)
    c21 = _add(m2, m4)
    c11 = _add(m1, m4)
    m3 = m(2)
    c22 = _add(c22, m3)
    m5 = m(4)
    c12 = _add(m3, m5)
    c11 = _sub(c11, m5)
    c22 = _add(c22, m(5))
    c11 = _add(c11, m(6))
    return [a + b for a, b in zip(c11, c12)] + [a + b for a, b in zip(c21, c22)]


def _join(blocks):
    return jnp.concatenate([jnp.concatenate(r, axis=1) for r in blocks], axis=0)


class _Pins:
    def __init__(self, zero, products, per_product):
        self.keep = lax.broadcasted_iota(jnp.int32, (8, 128), 0) >= zero
        self.points = [m[r:r + 8, 0:128] for m in products
                       for r in range(0, m.shape[0], m.shape[0] // per_product // 8 * 8)[:per_product]]

    def at(self, pos):
        return self.points[min(int(pos * len(self.points)), len(self.points) - 1)]

    def __call__(self, v, pos):
        point = self.at(pos)
        if v.dtype != f32:
            point = pltpu.bitcast(point, v.dtype)
        v = jnp.broadcast_to(v, (8, v.shape[1]))
        parts = [v[:, c:c + 128] for c in range(0, v.shape[1], 128)]
        return jnp.concatenate([jnp.where(self.keep, p, point) if p.shape[1] == 128 else p
                                for p in parts], axis=1)


def _no_pin(v, pos):
    return jnp.broadcast_to(v, (8, v.shape[1]))


def _rows(v8, n):
    return jnp.tile(v8, (n // 8, 1))


SCRATCH = dict(
    lead=((8 * 4, 128), f32), x_in=((D, S), bf16), wqkv_in=((D, 3 * D), bf16), wsq_in=((3, D, D), bf16), w3_in=((D, F), bf16),
    w4_in=((D, F), bf16), wqkv_s=((4, DQ // 2, 49 * 128), u32), wsq_s=((3, DHF // 2, 7 * DHP), u32),
    w3_s=((NU, 32, 49 * 128), u32), w4_s=((8, DHF // 2, FHF), u32),
    xa=((NB // 2, D, TB), f32), xb=((NB // 2, D, TB), f32), ya=((NB // 2, D, TB), f32), yb=((NB // 2, D, TB), f32),
    qa=((64, 49 * 128), u32), qb=((64, 49 * 128), u32),
    ra0=((DHP // 2, 7 * NT), u32), rb0=((DHP // 2, 7 * NT), u32), ra1=((DHP // 2, 7 * NT), u32),
    rb1=((DHP // 2, 7 * NT), u32), rg=((DHP // 2, 7 * NT), u32),
    ta=((7, FHF // 2, NT), u32), tb=((7, FHF // 2, NT), u32),
    qt=((D // 2, S), u32), qf=((H, 32, S), f32), kk=((H // HG, S // 4, 256), u32), kb=((DH, NV, 128), f32),
    vt=((H, 16, S), u32), ot=((D, S), f32),
    p0=((S // 2, QB), u32), p1=((S // 2, QB), u32), p2=((S // 2, QB), u32), p3=((S // 2, QB), u32),
    sbuf=((S, QB), f32), hbuf=((D, S + 256), f32), obuf=((D, S), bf16))


def _kernel(x_hbm, wqkv_hbm, wo_hbm, w1_hbm, w2_hbm, w3_hbm, w4_hbm, o_hbm, sems, *scratch):
    named = dict(zip(SCRATCH, scratch))
    (lead, x_in, wqkv_in, wsq_in, w3_in, w4_in, wqkv_s, wsq_s, w3_s, w4_s, xa, xb, ya, yb, qa, qb, ra0, rb0, ra1, rb1, rg,
     ta, tb, qt, qf, kk, kb, vt, ot, p0, p1, p2, p3, sbuf, hbuf, obuf) = [named[n] for n in SCRATCH]
    half_f = (NU + 1) // 2 * 256

    def x_copy(b):
        cols = pl.ds(pl.multiple_of(b * TB, TB), TB)
        return pltpu.make_async_copy(x_hbm.at[:, cols], x_in.at[:, cols], sems.at[b])

    def w_copies(it):
        cols = pl.ds(it * half_f, min(half_f, F - it * half_f))
        squares = ((wo_hbm, 0), (w1_hbm, 1)) if it == 0 else ((w2_hbm, 2),)
        return ([pltpu.make_async_copy(w, wsq_in.at[i], sems.at[NB + 1 + i]) for w, i in squares]
                + [pltpu.make_async_copy(w3_hbm.at[:, cols], w3_in.at[:, cols], sems.at[NB + 4 + it]),
                   pltpu.make_async_copy(w4_hbm.at[:, cols], w4_in.at[:, cols], sems.at[NB + 6 + it])])

    qkv_copy = pltpu.make_async_copy(wqkv_hbm, wqkv_in, sems.at[NB])
    for b in range(NB):
        x_copy(b).start()
    qkv_copy.start()

    def clear(i, _):
        rows = pl.ds(pl.multiple_of(i * 32, 32), 32)
        hbuf[rows, 0:TB + 256] = jnp.zeros((32, TB + 256), f32)
        hbuf[rows, S + 128:S + 256] = jnp.zeros((32, 128), f32)
        return 0

    lax.fori_loop(0, D // 32, clear, 0)

    def clear_scores(i, _):
        for r in (p0, p1, p2, p3):
            r[pl.ds(pl.multiple_of(i * 64, 64), 64), :] = jnp.zeros((64, QB), u32)
        return 0

    lax.fori_loop(0, S // 128, clear_scores, 0)
    for r in (ra0, rb0, ra1, rb1, rg):
        r[DHF // 2:, :] = jnp.zeros(((DHP - DHF) // 2, 7 * NT), u32)
    lead[0:8, :] = jnp.zeros((8, 128), f32)
    for r in (qa, qb):
        r[DQ // 2:, :] = jnp.zeros((64 - DQ // 2, 49 * 128), u32)

    def tile(i):
        return slice(i * 128, (i + 1) * 128)

    def tokens(b):
        return pl.ds(pl.multiple_of(b * TB, TB), TB)

    def prep_weight(load, dst, n, rows_out, scale=None):
        parts = []
        for j in range(n):
            w = load(slice(j * D // n, (j + 1) * D // n)).astype(f32)
            m = w.shape[1]
            if scale is not None:
                w = w * scale
            parts.append(jnp.concatenate([w, jnp.zeros(((512 - D) // n, m), f32)], axis=0).T)
        for j in range(m // (n * rows_out)):
            grid = [[p[(n * j + i) * rows_out:(n * j + i + 1) * rows_out] for p in parts] for i in range(n)]
            for i, t in enumerate(_lhs_terms(grid)):
                dst(j)[:, i * 512 // n:(i + 1) * 512 // n] = _pack(t)

    def put_rhs(dst, piece, pieces=7):
        n = 256 // dst.shape[0]
        step = D // n // pieces
        for k in range(pieces):
            rows = [piece(slice(i * D // n + k * step, i * D // n + (k + 1) * step), k) for i in range(n)]
            grid = [[x[:, c:c + TB // n] for c in range(0, TB, TB // n)] for x in rows]
            for i, t in enumerate(_rhs_terms(grid)):
                dst[k * step // 2:(k + 1) * step // 2, i * TB // n:(i + 1) * TB // n] = _pack(t)

    def matmul(w, base, rhs, z, chunks=None):
        n = 256 // rhs.shape[0]
        rows = pl.ds(pl.multiple_of(z * 8, 8), rhs.shape[0])
        issued, grids, lo = [], [], 0
        for size in chunks or (2 * w.shape[1],):
            part = slice(lo // 2, (lo + size) // 2)
            grids.append(_strassen(n, lambda i: _dot(_unpack(w[base, part, i * 512 // n:(i + 1) * 512 // n]),
                                                     _unpack(rhs[rows, i * TB // n:(i + 1) * TB // n])), issued))
            lo += size
        return _join([r for i in range(n) for r in (g[i] for g in grids)]), issued

    def ln_stats(load, s8, pin, lo, hi, n=4):
        mean = _colsum(s8) * (1.0 / D)
        step = D // n
        v8 = None
        for k in range(n):
            xc = load(slice(k * step, (k + 1) * step)) - _rows(pin(mean, lo + (hi - lo) * k / n), step)
            v8 = _rowsum8(xc * xc) if v8 is None else v8 + _rowsum8(xc * xc)
        var = _colsum(v8) * (1.0 / D)
        return mean, lax.rsqrt(var + EPS), var

    def ln_to_rhs(dst, load1, load2, s8, pin, lo, hi, n=7):
        mid = lo + (hi - lo) * 0.4
        mean, rstd, _ = ln_stats(load1, s8, pin, lo, mid)
        means = [pin(mean, mid + (hi - mid) * k / n) for k in range(n)]
        put_rhs(dst, lambda rows, k: (load2(rows) - _rows(means[k], rows.stop - rows.start)) * rstd, n)

    def first_ln(dst, xs, it, z1, z2, pin, lo, hi, n=4):
        mid = lo + (hi - lo) * 0.15
        step = D // n
        s8 = None
        for k in range(n):
            x = xs[it + z2, k * step:(k + 1) * step, :]
            x = jnp.concatenate([pin(x[0:8], lo + (mid - lo) * k / n), x[8:]], axis=0)
            s8 = _rowsum8(x) if s8 is None else s8 + _rowsum8(x)
        ln_to_rhs(dst, lambda rows: xs[it + z1, rows, :], lambda rows: xs[it + z2, rows, :], s8, pin, mid, hi)

    def o_to_rhs(dst, b, pin, lo, hi, n=7):
        ones = [pin(jnp.ones((8, TB), f32), lo + (hi - lo) * k / n) for k in range(n)]
        put_rhs(dst, lambda rows, k: ot[rows, tokens(b)] * _rows(ones[k], rows.stop - rows.start), n)

    def shifted_to_rhs(dst, b, pin, lo, hi):
        n = 14
        keeps = [pin(jnp.ones((8, 128), jnp.int32), lo + (hi - lo) * k / n) for k in range(n)]

        def piece(rows, k):
            sh = (1, -1, 2, -2)[rows.start // C4]
            w = hbuf[rows, pl.ds(pl.multiple_of(b * TB, TB), TB + 256)]
            g = w[:, 128 - sh:128 - sh + TB]
            return jnp.where(jnp.tile(keeps[k], (g.shape[0] // 8, TB // 128)) == 1, g, 0.0)
        put_rhs(dst, piece, n)

    def convert(it, _):
        for b, xs in ((2 * it, xa), (2 * it + 1, xb)):
            x_copy(b).wait()
            xs[it] = x_in[:, tokens(b)].astype(f32)
        return 0

    lax.fori_loop(0, NB // 2, convert, 0)
    first_ln(qa, xa, 0, 0, 0, _no_pin, 0.0, 1.0)
    qkv_copy.wait()
    for it in range(2):
        for c in w_copies(it):
            c.start()
    prep_weight(lambda rows: wqkv_in[rows, :], lambda j: wqkv_s.at[j], 4, DQ)

    def window(x, h):
        r0 = (DH * h) // 8 * 8
        return x[r0:r0 + 32, :]

    def lane_tiles_max(x):
        out = x[:, 0:128]
        for c in range(128, x.shape[1], 128):
            out = jnp.maximum(out, x[:, c:c + 128])
        return out

    def max_norm2(x):
        sq = x * x
        out = None
        for h in range(H):
            n2 = _colsum(_rowsum8(window(sq, h)))
            out = n2 if out is None else jnp.maximum(out, n2)
        return lane_tiles_max(out)

    def project(b, odd, rhs, z, bounds):
        k, pk = matmul(wqkv_s, 1, rhs, z, KCH)
        for g in range(H // HG):
            kg = jnp.concatenate([k[g * GW:(g + 1) * GW, :], jnp.zeros((128 - GW, TB), f32)], axis=0)
            kk.at[g][pl.ds(pl.multiple_of(b // 2 * (TB // 2), TB // 2), TB // 2), tile(odd)] = _pack(kg.T)
        v, pv = matmul(wqkv_s, 2, rhs, z, VCH)
        row = lax.broadcasted_iota(jnp.int32, (8, TB), 0)
        for h in range(H):
            w = window(v, h)
            if h % 2 == 0:
                w = jnp.concatenate([w[0:24], jnp.where(row < 4, w[24:32], 1.0)], axis=0)
            else:
                w = jnp.concatenate([jnp.where(row >= 4, w[0:8], 1.0), w[8:32]], axis=0)
            vt.at[h][:, tokens(b)] = _pack(w)
        q, pq = matmul(wqkv_s, 0, rhs, z, QCH)
        q = q * QSCALE
        qt[:, tokens(b)] = _pack(q)
        for h in range(H):
            w = window(q, h)
            if h % 2:
                w = jnp.concatenate([jnp.where(row < 4, pltpu.roll(w[24:32], 4, 0), w[0:8]), w[8:32]], axis=0)
            qf.at[h][:, tokens(b)] = w
        v_abs = lane_tiles_max(jnp.max(jnp.abs(v).reshape(D // 8, 8, TB), axis=0))
        bounds = (jnp.maximum(bounds[0], max_norm2(q)), jnp.maximum(bounds[1], max_norm2(k)),
                  jnp.maximum(bounds[2], v_abs))
        return _Pins(z, pk + pv + pq, 1), bounds

    def keys(h, lo, n):
        block, row = lo // TB, lo % TB
        return _unpack(kk[h // HG, (block // 2 * TB + row) // 2:(block // 2 * TB + row + n) // 2, tile(block % 2)])

    def spread_keys(h, groups, pin):
        for r0, pos in groups:
            half = r0 // 2
            if not isinstance(r0, int):
                r0, half = pl.multiple_of(r0, 16), pl.multiple_of(half, 8)
            kf = _unpack(kk[h // HG, pl.ds(half, 8), 0:128]).astype(f32)
            if not isinstance(h, int):
                odd = h % 2
                kf = pltpu.roll(kf, (128 + 4 * odd - DH * (h % HG)) % 128, 1)
                lane = lax.broadcasted_iota(jnp.int32, kf.shape, 1)
                kf = jnp.where(lane < 4 * odd, pltpu.roll(kf, 128 - DH, 1), kf)
            for d in range(DH):
                if d % 7 == 0:
                    kp = jnp.concatenate([pin(kf[0:8], pos(d)), pin(kf[8:16], pos(d))], axis=0)
                kb.at[d][pl.ds(r0, 16), :] = jnp.broadcast_to(kp[:, d:d + 1], (16, 128))

    def prep_unit(u):
        cols = pl.ds(pl.multiple_of(u * 256, 256), 256)
        prep_weight(lambda rows: w3_in[rows, cols], lambda j: w3_s.at[u], 4, 64)
        w = w4_in[:, cols].astype(f32) * 0.5
        terms = _lhs_terms([[w[:DHF, :128], w[:DHF, 128:]], [w[DHF:, :128], w[DHF:, 128:]]])
        for i, t in enumerate(terms):
            w4_s.at[i][:, pl.ds(pl.multiple_of(u * 128, 128), 128)] = _pack(t)

    def qkv_iter(it, bounds):
        z1, z2 = lax.shift_right_logical(it, 8), lax.shift_right_logical(it, 9)
        nxt = jnp.minimum(it + 1, NB // 2 - 1)
        pin, bounds = project(2 * it, 0, qa, z1, bounds)
        first_ln(qb, xb, it, z1, z2, pin, 0.0, 0.9)
        pin, bounds = project(2 * it + 1, 1, qb, z1, bounds)
        first_ln(qa, xa, nxt, z1, z2, pin, 0.0, 0.6)
        spread_keys(0, [(it * (NV // 2) + r0, lambda d, r0=r0: 0.55 + 0.8 * (r0 + 16 * d / DH) / NV)
                        for r0 in range(0, NV // 2, 16)], pin)
        return bounds

    def finish_head(acc, hp, qbp):
        odd = hp % 2
        l = jnp.where(odd == 1, acc[0:1, :], acc[28:29, :])
        o = acc * (1.0 / l)
        r0 = pl.multiple_of((DH * hp) // 8 * 8, 8)
        cols = pl.ds(qbp * QB if isinstance(qbp, int) else pl.multiple_of(qbp * QB, QB), QB)
        row = lax.broadcasted_iota(jnp.int32, (8, QB), 0)
        ot[pl.ds(r0, 8), cols] = jnp.where(row >= 4 * odd, o[0:8], ot[pl.ds(r0, 8), cols])
        ot[pl.ds(r0 + 8, 24), cols] = o[8:32]

    def masked_q(h, cols):
        qg = qt[pl.ds(pl.multiple_of((h // HG) * (GW // 2), 8), GW // 2), cols]
        row = lax.broadcasted_iota(jnp.int32, (GW // 2, QB), 0)
        lo = (h % HG) * (DH // 2)
        qm = jnp.where((row >= lo) & (row < lo + DH // 2), qg, jnp.zeros_like(qg))
        return _unpack(jnp.concatenate([qm, jnp.zeros(((128 - GW) // 2, QB), u32)], axis=0))

    def attn_head(h, last=False):
        hp = jnp.maximum(h - 1, 0)
        products = []
        for u, pbuf in enumerate((p0, p1, p2, p3)):
            cols = slice(u * QB, (u + 1) * QB)
            qm = None if last else masked_q(h, cols)
            acc = None
            for c in range(NC):
                lo, hi = max(c * KC, NV), (c + 1) * KC
                p = _unpack(pbuf[c * KC // 2:hi // 2, :])
                if hi > lo and not last:
                    st = _dot(keys(h, lo, hi - lo), qm)
                    pbuf[lo // 2:hi // 2, :] = _pack(jnp.exp2(st))
                    products += [st[r:r + 32] for r in range(0, hi - lo, 32)]
                d = _dot(_unpack(vt[hp, :, c * KC:hi]), p)
                products.append(d)
                acc = d if acc is None else acc + d
            finish_head(acc, hp, u)
        pin = _Pins(lax.shift_right_logical(h, 10), products, 4)
        if last:
            return pin
        units = [(u, r0, t0) for u in range(NQ) for r0 in range(0, NV, 16) for t0 in (0, 2)]

        def pos(n, d):
            return (n + d / DH) / len(units) * 0.99 - 0.015

        for n, (u, r0, t0) in enumerate(units):
            acc = {}
            for d in range(DH):
                ks = [kb[d, r:r + 8, :] for r in (r0, r0 + 8)]
                if d % 4 == 0 and pos(n, d) >= 0:
                    ks = [pin(k, pos(n, d)) for k in ks]
                for t in (t0, t0 + 1):
                    q = jnp.broadcast_to(qf[h, d:d + 1, tile(u * (QB // 128) + t)], (8, 128))
                    for r in range(2):
                        acc[r, t] = ks[r] * q if d == 0 else acc[r, t] + ks[r] * q
            for t in (t0, t0 + 1):
                st = jnp.concatenate([acc[0, t], acc[1, t]], axis=0)
                (p0, p1, p2, p3)[u][r0 // 2:r0 // 2 + 8, t * 128:(t + 1) * 128] = _pack(jnp.exp2(st))
        done = {r0: n + 1 for n, (u, r0, t0) in enumerate(units)}
        spread_keys(jnp.minimum(h + 1, H - 1), [(r0, lambda d, n=n: pos(n, d)) for r0, n in done.items()], pin)
        return pin

    def attn_guarded(i, _):
        h, cols = i // NQ, pl.ds(pl.multiple_of((i % NQ) * QB, QB), QB)
        qm = masked_q(h, cols)

        def scores(c, m):
            rows = pl.ds(pl.multiple_of(c * (KC // 2), KC // 2), KC // 2)
            first = c // (TB // KC) * 2 * TB + c % (TB // KC) * KC
            for odd in range(2):
                st = _dot(_unpack(kk[h // HG, rows, tile(odd)]), qm)
                sbuf[pl.ds(pl.multiple_of(first + odd * TB, KC), KC), :] = st
                m = jnp.maximum(m, jnp.max(st, axis=0, keepdims=True))
            return m

        m = lax.fori_loop(0, NC // 2, scores, jnp.full((1, QB), -jnp.inf, f32))

        def weighted(c, acc):
            rows = pl.ds(pl.multiple_of(c * KC, KC), KC)
            return acc + _dot(_unpack(vt[h, :, rows]), jnp.exp2(sbuf[rows, :] - m).astype(bf16))

        finish_head(lax.fori_loop(0, NC, weighted, jnp.zeros((32, QB), f32)), h, i % NQ)
        return 0

    def mix1_iter(it, _):
        z1, z2 = lax.shift_right_logical(it, 8), lax.shift_right_logical(it, 9)
        nxt = jnp.minimum(it + 1, NB // 2 - 1)

        def add_out_proj(xs, rhs):
            a, products = matmul(wsq_s, 0, rhs, z1)
            x = xs[it] + a
            xs[it] = x
            return _rowsum8(x), _Pins(z1, products, 4)

        def two_norms(dst, xs, ys, s8, pin, n=7):
            mean, rstd, var = ln_stats(lambda rows: xs[it + z1, rows, :], s8, pin, 0.0, 0.3)
            rstd2 = lax.rsqrt(var * rstd * rstd + EPS)
            means = [pin(mean, 0.35 + 0.55 * k / n) for k in range(n)]

            def piece(rows, k):
                y = (xs[it + z2, rows, :] - _rows(means[k], rows.stop - rows.start)) * rstd
                ys.at[it][rows, :] = y
                return y * rstd2
            put_rhs(dst, piece, n)

        def hidden(b, rhs):
            h, products = matmul(wsq_s, 1, rhs, z1)
            hbuf[:, pl.ds(pl.multiple_of(b * TB + 128, 128), TB)] = _gelu2(h)
            return _Pins(z1, products, 4)

        sa, pin = add_out_proj(xa, ra0)
        o_to_rhs(rb0, 2 * it + 1, pin, 0.0, 0.45)
        shifted_to_rhs(rg, 0, pin, 0.45, 0.98)
        sb, pin = add_out_proj(xb, rb0)
        two_norms(ra1, xa, ya, sa, pin)
        pin = hidden(2 * it, ra1)
        two_norms(rb1, xb, yb, sb, pin)
        pin = hidden(2 * it + 1, rb1)
        o_to_rhs(ra0, 2 * nxt, pin, 0.0, 0.3)
        return 0

    def mix2_iter(it, _):
        z1, z2 = lax.shift_right_logical(it, 8), lax.shift_right_logical(it, 9)
        nxt = jnp.minimum(it + 1, NB // 2 - 1)

        def add_mixer(ys, rhs):
            a, products = matmul(wsq_s, 2, rhs, z1)
            x1 = ys[it] + a
            ys[it] = x1
            return _rowsum8(x1), _Pins(z1, products, 4)

        def norm(dst, ys, s8, pin):
            ln_to_rhs(dst, lambda rows: ys[it + z1, rows, :], lambda rows: ys[it + z2, rows, :],
                      s8, pin, 0.0, 0.8)

        def up(dst, rhs):
            pins = []
            for u in range(NU):
                t, issued = matmul(w3_s, u, rhs, z1, UCH)
                t = _gelu2(t)
                halves = [[t[:128, :NT], t[:128, NT:]], [t[128:, :NT], t[128:, NT:]]]
                for i, term in enumerate(_rhs_terms(halves)):
                    dst.at[i][u * 64:(u + 1) * 64, :] = _pack(term)
                pins += issued[0:14]
            return _Pins(z1, pins, 1)

        def down(b, xs, ys, rhs):
            products = []
            a = _join(_strassen(2, lambda i: _dot(_unpack(w4_s[i]), _unpack(rhs[i + z1])), products))
            x = xs[it] + (ys[it + z1] + a)
            xs[it] = x
            obuf[:, tokens(b)] = x.astype(bf16)
            return _Pins(z1, products, 4)

        sa, pin = add_mixer(ya, rg)
        shifted_to_rhs(rb0, 2 * it + 1, pin, 0.0, 0.8)
        sb, pin = add_mixer(yb, rb0)
        norm(qa, ya, sa, pin)
        pin = up(ta, qa)
        norm(qb, yb, sb, pin)
        up(tb, qb)
        pin = down(2 * it, xa, ya, ta)
        shifted_to_rhs(rg, 2 * nxt, pin, 0.0, 0.9)
        pin = down(2 * it + 1, xb, yb, tb)
        first_ln(qa, xa, 0, z1, z2, pin, 0.0, 0.8)
        return 0

    def layer(l, carry):
        with jax.named_scope('qkv'):
            zeros = (jnp.zeros((1, 128), f32), jnp.zeros((1, 128), f32), lead[0:8, :])
            q2, k2, v1 = lax.fori_loop(0, NB // 2, qkv_iter, zeros)

        @pl.when(l == 0)
        def _():
            for j in range(2):
                for c in w_copies(j):
                    c.wait()

            def square(i, _):
                prep_weight(lambda rows: wsq_in[i, rows, :], lambda j: wsq_s.at[i], 2, DHF, jnp.where(i == 2, 0.5, 1.0))
                return 0

            def unit(u, _):
                prep_unit(u)
                return 0

            lax.fori_loop(0, 3, square, 0)
            lax.fori_loop(0, NU, unit, 0)

        small = jnp.logical_and(jnp.max(q2) * jnp.max(k2) <= SCORE_BOUND ** 2, jnp.max(v1) <= VALUE_BOUND)

        @pl.when(small)
        def _():
            with jax.named_scope('attn'):
                lax.fori_loop(0, H, lambda h, c: (attn_head(h), c)[1], 0)
            o_to_rhs(ra0, 0, attn_head(l * 0 + H, last=True), 0.3, 0.9)

        @pl.when(jnp.logical_not(small))
        def _():
            lax.fori_loop(0, H * NQ, attn_guarded, 0)
            o_to_rhs(ra0, 0, _no_pin, 0.0, 1.0)

        with jax.named_scope('mix1'):
            lax.fori_loop(0, NB // 2, mix1_iter, 0)
        with jax.named_scope('mix2'):
            lax.fori_loop(0, NB // 2, mix2_iter, 0)
        return carry

    with jax.named_scope('layers'):
        lax.fori_loop(0, 2, layer, 0)

    cp = pltpu.make_async_copy(obuf, o_hbm, sems.at[0])
    cp.start()
    cp.wait()


@jax.jit
def pallas_interleave_layers__mha_block__mixer_s_mlp__prompt_kernel(
        A_x, A_wqkv, A_wo, B_x, B_w1, B_w2, B_w3, B_w4):
    del B_x
    vmem = pltpu.VMEM
    hbm = pl.BlockSpec(memory_space=pltpu.HBM)
    out = pl.pallas_call(
        _kernel,
        out_shape=jax.ShapeDtypeStruct((D, S), A_x.dtype),
        in_specs=[hbm] * 7,
        out_specs=hbm,
        scratch_shapes=[pltpu.SemaphoreType.DMA((NB + 8,))] + [vmem(*v) for v in SCRATCH.values()],
        compiler_params=pltpu.CompilerParams(vmem_limit_bytes=110 * 2 ** 20),
    )(A_x.reshape(S, D).T, A_wqkv, A_wo, B_w1, B_w2, B_w3, B_w4.T)
    return out.T.reshape(1, S, D)
```

```python
import math

import jax
import jax.numpy as jnp
from jax import lax
from jax.experimental import pallas as pl
from jax.experimental.pallas import tpu as pltpu

S = 2048
D = 448
H = 16
DH = D // H
F = 1792
DHF = D // 2
DHP = 256
FHF = F // 2
DQ = D // 4
NT = 256
TB = 2 * NT
NB = S // TB
NU = F // 256
QB = 512
NQ = S // QB
KC = 128
NC = S // KC
HG = 4
GW = HG * DH
C4 = D // 4
T = {}
NV = T.get('NV', 224)
SCORE_BOUND = 60.0
VALUE_BOUND = 2.0 ** 40
EPS = 1e-5
QSCALE = (DH ** -0.5) * math.log2(math.e)

f32 = jnp.float32
bf16 = jnp.bfloat16
u32 = jnp.uint32


def _pack(x):
    return pltpu.bitcast(x.astype(bf16), u32)


def _unpack(x):
    return pltpu.bitcast(x, bf16)


def _rowsum8(x):
    return jnp.sum(x.reshape(x.shape[0] // 8, 8, x.shape[1]), axis=0)


def _colsum(x8):
    return jnp.sum(x8, axis=0, keepdims=True)


def _gelu2(x):
    c = math.sqrt(2.0 / math.pi)
    return x + x * jnp.tanh(x * (c + (c * 0.044715) * (x * x)))


def _dot(a, b):
    return jnp.dot(a, b, preferred_element_type=f32)


def _split(blocks):
    n = len(blocks) // 2
    return ([r[:n] for r in blocks[:n]], [r[n:] for r in blocks[:n]],
            [r[:n] for r in blocks[n:]], [r[n:] for r in blocks[n:]])


def _add(x, y):
    return [[a + b for a, b in zip(r, s)] for r, s in zip(x, y)]


def _sub(x, y):
    return [[a - b for a, b in zip(r, s)] for r, s in zip(x, y)]


def _lhs_terms(blocks):
    if len(blocks) == 1:
        return [blocks[0][0]]
    a11, a12, a21, a22 = _split(blocks)
    terms = (_add(a11, a22), _add(a21, a22), a11, a22, _add(a11, a12), _sub(a21, a11), _sub(a12, a22))
    return [t for x in terms for t in _lhs_terms(x)]


def _rhs_terms(blocks):
    if len(blocks) == 1:
        return [blocks[0][0]]
    b11, b12, b21, b22 = _split(blocks)
    terms = (_add(b11, b22), b11, _sub(b12, b22), _sub(b21, b11), b22, _add(b11, b12), _add(b21, b22))
    return [t for x in terms for t in _rhs_terms(x)]


def _strassen(n, prod, issued, base=0):
    if n == 1:
        issued.append(prod(base))
        return [[issued[-1]]]
    stride = 7 ** (n.bit_length() - 2)

    def m(i):
        return _strassen(n // 2, prod, issued, base + i * stride)

    m1 = m(0)
    m2 = m(1)
    c22 = _sub(m1, m2)
    m4 = m(3)
    c21 = _add(m2, m4)
    c11 = _add(m1, m4)
    m3 = m(2)
    c22 = _add(c22, m3)
    m5 = m(4)
    c12 = _add(m3, m5)
    c11 = _sub(c11, m5)
    c22 = _add(c22, m(5))
    c11 = _add(c11, m(6))
    return [a + b for a, b in zip(c11, c12)] + [a + b for a, b in zip(c21, c22)]


def _join(blocks):
    return jnp.concatenate([jnp.concatenate(r, axis=1) for r in blocks], axis=0)


def _in_ready_order(x, chunks):
    half_r, half_c, lo = x.shape[0] // 2, x.shape[1] // 2, 0
    n = x.shape[0] // sum(chunks)
    for size in chunks:
        for i, j in ((1, 0), (0, 1), (1, 1), (0, 0)):
            for q in range(n // 2):
                r0 = i * half_r + q * sum(chunks) + lo
                yield slice(r0, r0 + size), slice(j * half_c, (j + 1) * half_c)
        lo += size


class _Pins:
    def __init__(self, zero, products, per_product):
        self.keep = lax.broadcasted_iota(jnp.int32, (8, 128), 0) >= zero
        self.points = [m[r:r + 8, 0:128] for m in products
                       for r in range(0, m.shape[0], max(m.shape[0] // per_product // 8, 1) * 8)[:per_product]]

    def at(self, pos):
        return self.points[min(int(pos * len(self.points)), len(self.points) - 1)]

    def __call__(self, v, pos):
        point = self.at(pos)
        if v.dtype != f32:
            point = pltpu.bitcast(point, v.dtype)
        v = jnp.broadcast_to(v, (8, v.shape[1]))
        parts = [v[:, c:c + 128] for c in range(0, v.shape[1], 128)]
        return jnp.concatenate([jnp.where(self.keep, p, point) if p.shape[1] == 128 else p
                                for p in parts], axis=1)


def _no_pin(v, pos):
    return jnp.broadcast_to(v, (8, v.shape[1]))


def _rows(v8, n):
    return jnp.tile(v8, (n // 8, 1))


SCRATCH = dict(
    x_in=((D, S), bf16), wqkv_in=((D, 3 * D), bf16), wsq_in=((3, D, D), bf16), w3_in=((D, F), bf16),
    w4_in=((D, F), bf16), wqkv_s=((4, DQ // 2, 49 * 128), u32), wsq_s=((3, DHF // 2, 7 * DHP), u32),
    w3_s=((NU, 32, 49 * 128), u32), w4_s=((49, DQ // 2, 512), u32), w4_t=((8, DHF // 2, FHF), u32),
    xa=((NB // 2, D, TB), f32), xb=((NB // 2, D, TB), f32), ya=((NB // 2, D, TB), f32), yb=((NB // 2, D, TB), f32),
    qa=((64, 49 * 128), u32), qb=((64, 49 * 128), u32),
    ra0=((DHP // 2, 7 * NT), u32), rb0=((DHP // 2, 7 * NT), u32), ra1=((DHP // 2, 7 * NT), u32),
    rb1=((DHP // 2, 7 * NT), u32), rg=((DHP // 2, 7 * NT), u32),
    ta=((7, FHF // 2, NT), u32), tf=((F, TB), f32), tb=((192, 49 * 128), u32), sb=((64, 7 * NT), u32),
    qt=((D // 2, S), u32), qf=((H, 32, S), f32), kk=((H // HG, S // 4, 256), u32), kb=((32, NV, 128), f32), kf=((2 * H, 32, 256), f32),
    vt=((H, 16, S), u32), ot=((D, S), f32),
    pbuf=((NQ, S // 2, QB), u32),
    sbuf=((S, QB), f32), hbuf=((D, S + 256), f32), obuf=((D, S), bf16))


def _kernel(x_hbm, wqkv_hbm, wo_hbm, w1_hbm, w2_hbm, w3_hbm, w4_hbm, o_hbm, sems, *scratch):
    named = dict(zip(SCRATCH, scratch))
    (x_in, wqkv_in, wsq_in, w3_in, w4_in, wqkv_s, wsq_s, w3_s, w4_s, w4_t, xa, xb, ya, yb, qa, qb, ra0, rb0, ra1, rb1, rg,
     ta, tf, tb, sb, qt, qf, kk, kb, kf, vt, ot, pbuf, sbuf, hbuf, obuf) = [named[n] for n in SCRATCH]
    def x_copy(b):
        cols = pl.ds(b * TB, TB)
        return pltpu.make_async_copy(x_hbm.at[:, cols], x_in.at[:, cols], sems.at[b])

    def out_copy(b):
        cols = pl.ds(pl.multiple_of(b * TB, TB), TB)
        return pltpu.make_async_copy(obuf.at[:, cols], o_hbm.at[:, cols], sems.at[b])

    w_copies = [pltpu.make_async_copy(src, dst, sems.at[NB + 1 + i]) for i, (src, dst) in enumerate((
        (wo_hbm, wsq_in.at[0]), (w1_hbm, wsq_in.at[1]), (w2_hbm, wsq_in.at[2]), (w3_hbm, w3_in), (w4_hbm, w4_in)))]
    qkv_copies = [pltpu.make_async_copy(wqkv_hbm.at[pl.ds(j * DQ, DQ)], wqkv_in.at[pl.ds(j * DQ, DQ)],
                                        sems.at[NB + 6 + j]) for j in range(4)]
    x_copy(0).start()
    for c in qkv_copies:
        c.start()
    for b in range(1, NB):
        x_copy(b).start()

    hbuf[:, 0:128] = jnp.zeros((D, 128), f32)
    hbuf[:, S + 128:S + 256] = jnp.zeros((D, 128), f32)
    for r in (ra0, rb0, ra1, rb1, rg):
        r[DHF // 2:, :] = jnp.zeros(((DHP - DHF) // 2, 7 * NT), u32)
    for r in (qa, qb):
        r[DQ // 2:, :] = jnp.zeros((64 - DQ // 2, 49 * 128), u32)

    def tile(i):
        return slice(i * 128, (i + 1) * 128)

    def tokens(b):
        return pl.ds(pl.multiple_of(b * TB, TB), TB)

    def prep_weight(load, dst, n, rows_out, pin, lo, hi):
        parts = []
        mid = lo + (hi - lo) * 0.4
        for j in range(n):
            w = load(slice(j * D // n, (j + 1) * D // n)).astype(f32)
            m = w.shape[1]
            w = jnp.concatenate([pin(w[0:8], lo + (mid - lo) * j / n), w[8:], jnp.zeros(((512 - D) // n, m), f32)], axis=0)
            parts.append(w.T)
        for j in range(m // (n * rows_out)):
            for r in range(0, rows_out, 16):
                grid = [[p[(n * j + i) * rows_out + r:(n * j + i) * rows_out + r + 16] for p in parts] for i in range(n)]
                if pin is not _no_pin:
                    pos = mid + (hi - mid) * r / rows_out
                    grid = [[jnp.concatenate([pin(x[0:8], pos), pin(x[8:16], pos)], axis=0) for x in g] for g in grid]
                for i, t in enumerate(_lhs_terms(grid)):
                    dst(j)[r // 2:r // 2 + 8, i * 512 // n:(i + 1) * 512 // n] = _pack(t)
        return parts

    def rhs_terms(grid, pin, pos):
        if len(grid) == 2:
            return _rhs_terms(grid)
        b11, b12, b21, b22 = _split(grid)

        def late(blocks, j):
            return [[jnp.concatenate([pin(x[0:8], pos((j + 1) / 8)), pin(x[8:16], pos((j + 1) / 8))], axis=0)
                     for x in r] for r in blocks]
        outer = (_add(late(b11, 0), b22), late(b11, 1), _sub(late(b12, 2), b22), _sub(late(b21, 3), b11),
                 late(b22, 4), _add(late(b12, 5), b11), _add(late(b21, 6), b22))
        return [t for x in outer for t in _rhs_terms(x)]

    def put_rhs(dst, piece, pin=None, pos=None):
        n = 256 // dst.shape[0]
        for k in range(D // n // 16):
            rows = [piece(slice(i * D // n + k * 16, i * D // n + (k + 1) * 16), k) for i in range(n)]
            grid = [[x[:, c:c + TB // n] for c in range(0, TB, TB // n)] for x in rows]
            for i, t in enumerate(rhs_terms(grid, pin, lambda f: pos(k + f))):
                dst[k * 8:(k + 1) * 8, i * TB // n:(i + 1) * TB // n] = _pack(t)

    def matmul(w, base, rhs, z, chunks=None):
        n = 256 // rhs.shape[0]
        rows = pl.ds(pl.multiple_of(z * 8, 8), rhs.shape[0])
        issued, grids, lo = [], [], 0
        for size in chunks or (2 * w.shape[1],):
            part = slice(lo // 2, (lo + size) // 2)
            grids.append(_strassen(n, lambda i: _dot(_unpack(w[base, part, i * 512 // n:(i + 1) * 512 // n]),
                                                     _unpack(rhs[rows, i * TB // n:(i + 1) * TB // n])), issued))
            lo += size
        return _join([r for i in range(n) for r in (g[i] for g in grids)]), issued

    def update(ref, it, a, chunks, new):
        sums = {}
        for rows, cols in _in_ready_order(a, chunks):
            x = new(rows, cols, a[rows, cols])
            ref.at[it][rows, cols] = x
            sums[cols.start] = _rowsum8(x) + sums[cols.start] if cols.start in sums else _rowsum8(x)
        return jnp.concatenate([sums[0], sums[NT]], axis=1)

    def ln_stats(load, s8, pin, lo, hi, n=T.get('N', 14)):
        mean = _colsum(s8) * (1.0 / D)
        step = D // n
        v8 = None
        for k in range(n):
            xc = load(slice(k * step, (k + 1) * step)) - _rows(pin(mean, lo + (hi - lo) * k / n), step)
            v8 = _rowsum8(xc * xc) if v8 is None else v8 + _rowsum8(xc * xc)
        var = _colsum(v8) * (1.0 / D)
        return mean, lax.rsqrt(var + EPS), var

    def ln_to_rhs(dst, load1, load2, s8, pin, lo, hi, n=7):
        mid = lo + (hi - lo) * T.get('o', 0.4)
        mean, rstd, _ = ln_stats(load1, s8, pin, lo, mid)
        means = [pin(mean, mid + (hi - mid) * k / n) for k in range(n)]
        put_rhs(dst, lambda rows, k: (load2(rows) - _rows(means[k], 16)) * rstd,
                pin, lambda k: mid + (hi - mid) * k / n)

    def first_ln(dst, xs, it, z1, z2, pin, lo, hi, n=4):
        mid = lo + (hi - lo) * 0.15
        step = D // n
        s8 = None
        for k in range(n):
            x = xs[it + z2, k * step:(k + 1) * step, :]
            x = jnp.concatenate([pin(x[0:8], lo + (mid - lo) * k / n), x[8:]], axis=0)
            s8 = _rowsum8(x) if s8 is None else s8 + _rowsum8(x)
        ln_to_rhs(dst, lambda rows: xs[it + z1, rows, :], lambda rows: xs[it + z2, rows, :], s8, pin, mid, hi)

    def o_to_rhs(dst, b, pin, lo, hi, n=14):
        ones = [pin(jnp.ones((8, TB), f32), lo + (hi - lo) * k / n) for k in range(n)]
        put_rhs(dst, lambda rows, k: ot[rows, tokens(b)] * _rows(ones[k], 16))

    def shifted_to_rhs(dst, b, pin, lo, hi, valid=1):
        n = 14
        keeps = [pin(jnp.full((8, 128), valid, jnp.int32), lo + (hi - lo) * k / n) for k in range(n)]

        def piece(rows, k):
            sh = (1, -1, 2, -2)[rows.start // C4]
            w = hbuf[rows, pl.ds(pl.multiple_of(b * TB, TB), TB + 256)]
            g = w[:, 128 - sh:128 - sh + TB]
            return jnp.where(jnp.tile(keeps[k], (g.shape[0] // 8, TB // 128)) == 1, g, 0.0)
        put_rhs(dst, piece)

    def convert(b):
        x_copy(b).wait()
        (xa, xb)[b % 2][b // 2] = x_in[:, b * TB:(b + 1) * TB].astype(f32)

    def qkv_rows(rows):
        qkv_copies[rows.start // DQ].wait()
        return wqkv_in[rows, :]

    convert(0)
    first_ln(qa, xa, 0, 0, 0, _no_pin, 0.0, 1.0)
    parts = prep_weight(qkv_rows, lambda j: wqkv_s.at[j], 4, DQ, _no_pin, 0.0, 1.0)
    v_max = D * jnp.max(jnp.abs(jnp.concatenate([p[2 * D:] for p in parts], axis=0)))
    for c in w_copies:
        c.start()
    for b in range(1, NB):
        convert(b)

    def window(x, h):
        r0 = (DH * h) // 8 * 8
        return x[r0:r0 + 32, :]

    def head_rows(x, h):
        w = window(x, h)
        if h % 2:
            row = lax.broadcasted_iota(jnp.int32, (8, x.shape[1]), 0)
            w = jnp.concatenate([jnp.where(row < 4, pltpu.roll(w[24:32], 4, 0), w[0:8]), w[8:32]], axis=0)
        return w

    def lane_tiles_max(x):
        out = x[:, 0:128]
        for c in range(128, x.shape[1], 128):
            out = jnp.maximum(out, x[:, c:c + 128])
        return out

    def max_norm2(x):
        sq = x * x
        out = None
        for h in range(HG):
            n2 = _colsum(_rowsum8(window(sq, h)))
            out = n2 if out is None else jnp.maximum(out, n2)
        return lane_tiles_max(out)

    def project(b, odd, rhs, z, bounds):
        def ready(x):
            for rows, cols in _in_ready_order(x, (DQ,)):
                yield rows.start // DQ, x[rows, cols], cols.start

        def at(t0):
            return pl.ds(pl.multiple_of(b * TB + t0, NT), NT)

        q2, k2 = bounds
        k, pk = matmul(wqkv_s, 1, rhs, z)
        for g, x, t0 in ready(k):
            kg = jnp.concatenate([x, jnp.zeros((128 - GW, NT), f32)], axis=0)
            rows = pl.ds(pl.multiple_of((b // 2 * TB + t0) // 2, NT // 2), NT // 2)
            kk.at[g][rows, tile(odd)] = _pack(kg.T)
            k2 = jnp.maximum(k2, max_norm2(x))
            if not odd and t0 == 0:
                for j in range(HG):
                    kf.at[b // 2 * H + g * HG + j][...] = head_rows(x, j)
        v, pv = matmul(wqkv_s, 2, rhs, z)
        row = lax.broadcasted_iota(jnp.int32, (8, NT), 0)
        for g, x, t0 in ready(v):
            for j in range(HG):
                w = window(x, j)
                if j % 2 == 0:
                    w = jnp.concatenate([w[0:24], jnp.where(row < 4, w[24:32], 1.0)], axis=0)
                else:
                    w = jnp.concatenate([jnp.where(row >= 4, w[0:8], 1.0), w[8:32]], axis=0)
                vt.at[g * HG + j][:, at(t0)] = _pack(w)
        q, pq = matmul(wqkv_s, 0, rhs, z)
        for g, x, t0 in ready(q):
            x = x * QSCALE
            qt[g * GW // 2:(g + 1) * GW // 2, at(t0)] = _pack(x)
            q2 = jnp.maximum(q2, max_norm2(x))
            for j in range(HG):
                qf.at[g * HG + j][:, at(t0)] = head_rows(x, j)
        return _Pins(z, pk + pv + pq, 1), (q2, k2)

    def keys(h, lo, n):
        block, row = lo // TB, lo % TB
        return _unpack(kk[h // HG, (block // 2 * TB + row) // 2:(block // 2 * TB + row + n) // 2, tile(block % 2)])

    def spread_keys(h, t, pin, lo, hi):
        n = min(NV - 128 * t, 128)
        for d in range(DH):
            row = pin(kf[h, d:d + 1, tile(t)], lo + (hi - lo) * d / DH)
            kb.at[d][128 * t:128 * t + n, :] = _rows(row[:, 0:n], 128).T

    def prep_square(i, pin, lo, hi):
        prep_weight(lambda rows: wsq_in[i, rows, :], lambda j: wsq_s.at[i], 2, DHF, pin, lo, hi)

    def prep_up(v, pin, lo, hi):
        for j in range(2):
            u = jnp.minimum(2 * v + j, NU - 1)
            prep_weight(lambda rows: w3_in[rows, pl.ds(pl.multiple_of(u * 256, 256), 256)], lambda _: w3_s.at[u],
                        4, 64, pin, lo + (hi - lo) * j / 2, lo + (hi - lo) * (j + 1) / 2)

    def prep_down2(p, _):
        low = lax.broadcasted_iota(jnp.int32, (16, 128), 1) < 64

        def piece(r, _):
            grid = []
            for i in range(4):
                rows = pl.ds(pl.multiple_of(i * DQ + r * 16, 16), 16)
                w = w4_in[rows, pl.ds(pl.multiple_of(p * 512, 512), 512)].astype(f32)
                t = [w[:, tile(c)] for c in range(4)]
                grid.append([jnp.where(low, t[0], pltpu.roll(t[2], 64, 1)), jnp.where(low, pltpu.roll(t[0], 64, 1), t[2]),
                             jnp.where(low, t[1], pltpu.roll(t[3], 64, 1)), jnp.where(low, pltpu.roll(t[1], 64, 1), t[3])])
            for i, term in enumerate(_lhs_terms(grid)):
                w4_s.at[i][pl.ds(pl.multiple_of(r * 8, 8), 8), pl.ds(pl.multiple_of(p * 128, 128), 128)] = _pack(term)
            return 0

        return lax.fori_loop(0, DQ // 16, piece, 0, unroll=True)

    def prep_down1(u, _):
        cols = pl.ds(pl.multiple_of(u * 256, 256), 256)
        for r in range(0, DHF, 32):
            top = w4_in[r:r + 32, cols].astype(f32)
            bot = w4_in[DHF + r:DHF + r + 32, cols].astype(f32)
            for i, t in enumerate(_lhs_terms([[top[:, :128], top[:, 128:]], [bot[:, :128], bot[:, 128:]]])):
                w4_t.at[i][r // 2:r // 2 + 16, pl.ds(pl.multiple_of(u * 128, 128), 128)] = _pack(t)
        return 0

    def qkv_iter(it, bounds):
        z1, z2 = lax.shift_right_logical(it, 8), lax.shift_right_logical(it, 9)
        nxt = jnp.minimum(it + 1, NB // 2 - 1)
        pin, bounds = project(2 * it, 0, qa, z1, bounds)
        first_ln(qb, xb, it, z1, z2, pin, T.get('m0', 0.0), T.get('m', 0.85))
        pin, bounds = project(2 * it + 1, 1, qb, z1, bounds)
        first_ln(qa, xa, nxt, z1, z2, pin, T.get('n0', 0.0), T.get('n', 0.75))
        return bounds

    def finish_head(acc, hp, qbp):
        odd = hp % 2
        l = jnp.where(odd == 1, acc[0:1, :], acc[28:29, :])
        o = acc * (1.0 / l)
        r0 = pl.multiple_of((DH * hp) // 8 * 8, 8)
        cols = pl.ds(qbp * QB if isinstance(qbp, int) else pl.multiple_of(qbp * QB, QB), QB)
        row = lax.broadcasted_iota(jnp.int32, (8, QB), 0)
        ot[pl.ds(r0, 8), cols] = jnp.where(row >= 4 * odd, o[0:8], ot[pl.ds(r0, 8), cols])
        ot[pl.ds(r0 + 8, 24), cols] = o[8:32]

    def masked_q(h, cols):
        g0 = (h // HG) * (GW // 2)
        qg = qt[pl.ds(g0 if isinstance(g0, int) else pl.multiple_of(g0, 8), GW // 2), cols]
        row = lax.broadcasted_iota(jnp.int32, (GW // 2, QB), 0)
        lo = (h % HG) * (DH // 2)
        qm = jnp.where((row >= lo) & (row < lo + DH // 2), qg, jnp.zeros_like(qg))
        return _unpack(jnp.concatenate([qm, jnp.zeros(((128 - GW) // 2, QB), u32)], axis=0))

    def attn_head(h, last=False):
        hp = h - 1
        products = []

        def weighted(u, c):
            d = _dot(_unpack(vt[hp, :, c * KC:(c + 1) * KC]), _unpack(pbuf[u, c * KC // 2:(c + 1) * KC // 2, :]))
            products.append(d)
            return d

        early = pl.cdiv(NV, KC)
        accs = [sum(weighted(u, c) for c in range(1, early)) + weighted(u, 0) for u in range(NQ)]
        for u in range(NQ):
            qm = None if last else masked_q(h, slice(u * QB, (u + 1) * QB))
            acc = accs[u]
            for c in range(NC):
                lo, hi = max(c * KC, NV), (c + 1) * KC
                if hi > lo and not last:
                    st = _dot(keys(h, lo, hi - lo), qm)
                    products += [st[r:r + 32] for r in range(0, hi - lo, 32)]
                if c >= early:
                    acc = acc + weighted(u, c)
                if hi > lo and not last:
                    pbuf.at[u][lo // 2:hi // 2, :] = _pack(jnp.exp2(st))
            finish_head(acc, hp, u)
        pin = _Pins(lax.shift_right_logical(h, 10), products, 4)
        if last:
            return pin
        units = [(u, r0, t0) for r0 in range(0, NV, 16) for u in range(NQ) for t0 in (0, 2)]

        def pos(n, d):
            return (n + d / DH) / len(units) * (T.get('A', 0.98) + T.get('B', 0.015)) - T.get('B', 0.015)

        spread_keys(h, 1, pin, 0.01, T.get('F', 0.35))
        for n, (u, r0, t0) in enumerate(units):
            acc = {}
            for d in range(DH):
                ks = [kb[d, r:r + 8, :] for r in (r0, r0 + 8)]
                if d % (T.get('C', 4) if r0 < 128 else T.get('C1', 4)) == 0 and pos(n, d) >= 0:
                    ks = [pin(k, pos(n, d)) for k in ks]
                for t in (t0, t0 + 1):
                    q = jnp.broadcast_to(qf[h, d:d + 1, tile(u * (QB // 128) + t)], (8, 128))
                    for r in range(2):
                        acc[r, t] = ks[r] * q if d == 0 else acc[r, t] + ks[r] * q
            for t in (t0, t0 + 1):
                st = jnp.concatenate([acc[0, t], acc[1, t]], axis=0)
                pbuf.at[u][r0 // 2:r0 // 2 + 8, t * 128:(t + 1) * 128] = _pack(jnp.exp2(st))
        done = {r0: n + 1 for n, (u, r0, t0) in enumerate(units)}
        nxt = jnp.minimum(h + 1, H - 1)
        spread_keys(nxt, 0, pin, pos(done[128 - 16], 0), T.get('E', 0.95))
        return pin

    def attn_first(u, _):
        qm = masked_q(0, pl.ds(pl.multiple_of(u * QB, QB), QB))
        products = []
        for c in range(NC):
            st = _dot(keys(0, c * KC, KC), qm)
            pbuf.at[u][c * KC // 2:(c + 1) * KC // 2, :] = _pack(jnp.exp2(st))
            products.append(st)
        pin = _Pins(lax.shift_right_logical(u, 10), products, 8)
        prep_up(u, pin, 0.0, T.get('G', 0.75))
        rows = kf[1, pl.ds(pl.multiple_of(8 * u, 8), 8), tile(0)]
        for d in range(8):
            kb.at[8 * u + d][0:128, :] = _rows(pin(rows[d:d + 1], T.get('G2', 0.75) + 0.12 * d / 8), 128).T
        return 0

    def attn_guarded(i, _):
        h, cols = i // NQ, pl.ds(pl.multiple_of((i % NQ) * QB, QB), QB)
        qm = masked_q(h, cols)

        def scores(c, m):
            rows = pl.ds(pl.multiple_of(c * (KC // 2), KC // 2), KC // 2)
            first = c // (TB // KC) * 2 * TB + c % (TB // KC) * KC
            for odd in range(2):
                st = _dot(_unpack(kk[h // HG, rows, tile(odd)]), qm)
                sbuf[pl.ds(pl.multiple_of(first + odd * TB, KC), KC), :] = st
                m = jnp.maximum(m, jnp.max(st, axis=0, keepdims=True))
            return m

        m = lax.fori_loop(0, NC // 2, scores, jnp.full((1, QB), -jnp.inf, f32))

        def weighted(c, acc):
            rows = pl.ds(pl.multiple_of(c * KC, KC), KC)
            return acc + _dot(_unpack(vt[h, :, rows]), jnp.exp2(sbuf[rows, :] - m).astype(bf16))

        finish_head(lax.fori_loop(0, NC, weighted, jnp.zeros((32, QB), f32)), h, i % NQ)
        return 0

    def mix1_iter(it, _):
        z1, z2 = lax.shift_right_logical(it, 8), lax.shift_right_logical(it, 9)
        nxt = jnp.minimum(it + 1, NB // 2 - 1)

        def add_out_proj(xs, rhs):
            chunks = T.get('S0', (DHF,))
            a, products = matmul(wsq_s, 0, rhs, z1, chunks)
            return update(xs, it, a, chunks, lambda r, c, v: xs[it, r, c] + v), _Pins(z1, products, 4)

        def two_norms(dst, xs, ys, s8, pin, n=14):
            mean, rstd, var = ln_stats(lambda rows: xs[it + z1, rows, :], s8, pin, 0.0, T.get('c', 0.2))
            rstd2 = lax.rsqrt(var * rstd * rstd + EPS)
            means = [pin(mean, T.get('d', 0.22) + (T.get('e', 0.75) - T.get('d', 0.22)) * k / n) for k in range(n)]

            def piece(rows, k):
                y = (xs[it + z2, rows, :] - _rows(means[k], rows.stop - rows.start)) * rstd
                ys.at[it][rows, :] = y
                return y * rstd2
            put_rhs(dst, piece)

        def hidden(b, rhs):
            chunks = T.get('S1', (DHF,))
            h, products = matmul(wsq_s, 1, rhs, z1, chunks)
            for rows, cols in _in_ready_order(h, chunks):
                hbuf[rows, pl.ds(pl.multiple_of(b * TB + 128 + cols.start, 128), NT)] = _gelu2(h[rows, cols])
            return _Pins(z1, products, 4)

        suma, pin = add_out_proj(xa, ra0)
        o_to_rhs(rb0, 2 * it + 1, pin, 0.0, T.get('a', 0.4))
        shifted_to_rhs(rg, 0, pin, T.get('a', 0.4), T.get('b', 0.9), valid=it)
        sumb, pin = add_out_proj(xb, rb0)
        two_norms(ra1, xa, ya, suma, pin)
        pin = hidden(2 * it, ra1)
        two_norms(rb1, xb, yb, sumb, pin)
        pin = hidden(2 * it + 1, rb1)
        o_to_rhs(ra0, 2 * nxt, pin, T.get('f', 0.0), T.get('g', 0.6))
        return 0

    def mix2_iter(it, _):
        z1, z2 = lax.shift_right_logical(it, 8), lax.shift_right_logical(it, 9)
        nxt = jnp.minimum(it + 1, NB // 2 - 1)

        def add_mixer(ys, rhs):
            chunks = T.get('S2', (112, 112))
            a, products = matmul(wsq_s, 2, rhs, z1, chunks)
            return update(ys, it, a, chunks, lambda r, c, v: ys[it, r, c] + 0.5 * v), _Pins(z1, products, 4)

        def norm(dst, ys, s8, pin, end):
            ln_to_rhs(dst, lambda rows: ys[it + z1, rows, :], lambda rows: ys[it + z2, rows, :],
                      s8, pin, 0.0, end)

        def up(rhs, put):
            pins = []
            for u in range(NU):
                t, issued = matmul(w3_s, u, rhs, z1, (32, 32))
                put(u, _gelu2(t))
                pins += issued[T.get('k0', 0):T.get('k', 49)]
            return _Pins(z1, pins, 1)

        def halves(t):
            return [[t[:128, :NT], t[:128, NT:]], [t[128:, :NT], t[128:, NT:]]]

        def put_a(u, t):
            for i, term in enumerate(_rhs_terms(halves(t))):
                ta.at[i][u * 64:(u + 1) * 64, :] = _pack(term)

        def put_b(u, t):
            tf[u * 256:(u + 1) * 256, :] = t

        def down_a():
            products, grids, lo = [], [], 0
            for size in T.get('D', (32,) * 7):
                part = slice(lo // 2, (lo + size) // 2)
                grids.append(_strassen(2, lambda i: _dot(_unpack(w4_t[i, part, :]), _unpack(ta[i + z1])), products))
                lo += size
            return _join([g[i] for i in range(2) for g in grids]), _Pins(z1, products, 8)

        def split_b(pin, end):
            def hidden(lo, n):
                return tf[pl.ds(pl.multiple_of(lo + z1 * 8, 8), n), :]

            for r in range(0, 128, 16):
                top, bot = hidden((NU - 1) * 256 + r, 16), hidden((NU - 1) * 256 + 128 + r, 16)
                top = jnp.concatenate([pin(top[0:8], end * (r / 128) / (4 * NU - 3)), top[8:]], axis=0)
                for i, term in enumerate(_rhs_terms([[top[:, :NT], top[:, NT:]], [bot[:, :NT], bot[:, NT:]]])):
                    sb[r // 2:r // 2 + 8, i * NT:(i + 1) * NT] = _pack(term)
            for k in range(4 * (NU - 1)):
                rows = [hidden(k // 4 * 256 + i * 64 + k % 4 * 16, 16) for i in range(4)]
                grid = [[x[:, tile(c)] for c in range(4)] for x in rows]
                for i, term in enumerate(rhs_terms(grid, pin, lambda f: end * (k + 1 + f) / (4 * NU - 3))):
                    tb[k * 8:(k + 1) * 8, tile(i)] = _pack(term)

        def down_b():
            tail = _join(_strassen(2, lambda i: _dot(
                _unpack(w4_t[i, :, tile(NU - 1)]),
                _unpack(sb[pl.ds(pl.multiple_of(z1 * 8, 8), 64), i * NT:(i + 1) * NT])), []))
            products, grids, lo = [], [], 0
            for size in T.get('D2', (48, 32, 32)):
                part = slice(lo // 2, (lo + size) // 2)
                grids.append(_strassen(4, lambda i: _dot(_unpack(w4_s[i, part, 0:384]),
                                                         _unpack(tb[pl.ds(pl.multiple_of(z1 * 8, 8), 192), tile(i)])), products))
                lo += size
            return _join([g[i] for i in range(4) for g in grids]) + tail, _Pins(z1, products, 1)

        def down(b, xs, ys, a, chunks):
            def new(rows, cols, v):
                x = xs[it, rows, cols] + (ys[it + z1, rows, cols] + 0.5 * v)
                obuf[rows, pl.ds(pl.multiple_of(b * TB + cols.start, NT), NT)] = x.astype(bf16)
                return x
            update(xs, it, a, chunks, new)
            out_copy(b).start()

        suma, pin = add_mixer(ya, rg)
        shifted_to_rhs(rb0, 2 * it + 1, pin, 0.0, T.get('j', 0.8))
        sumb, pin = add_mixer(yb, rb0)
        norm(qa, ya, suma, pin, T.get('h', 0.8))
        pin = up(qa, put_a)
        norm(qb, yb, sumb, pin, T.get('i', 0.8))
        up(qb, put_b)
        a, pin = down_a()
        down(2 * it, xa, ya, a, T.get('D', (32,) * 7))
        split_b(pin, T.get('p', 0.8))
        a, pin = down_b()
        down(2 * it + 1, xb, yb, a, T.get('D2', (48, 32, 32)))
        shifted_to_rhs(rg, 2 * nxt, pin, 0.0, T.get('q', 0.3))
        first_ln(qa, xa, 0, z1, z2, pin, T.get('q', 0.3), T.get('l', 0.95))
        return 0

    def layer(l, carry):
        zero = jnp.zeros((1, 128), f32)
        q2, k2 = lax.fori_loop(0, NB // 2, qkv_iter, (zero, zero))

        @pl.when(l == 0)
        def _():
            for c in w_copies:
                c.wait()
            lax.fori_loop(0, NU, prep_down1, 0)
            lax.fori_loop(0, NU // 2, prep_down2, 0)

        lax.fori_loop(0, NQ, attn_first, 0)
        small = jnp.logical_and(jnp.max(q2) * jnp.max(k2) <= SCORE_BOUND ** 2, v_max <= VALUE_BOUND)

        @pl.when(small)
        def _():
            lax.fori_loop(1, H, lambda h, c: (attn_head(h), c)[1], 0)
            pin = attn_head(l * 0 + H, last=True)
            end = T.get('H', 0.66)
            for i in range(3):
                prep_square(i, pin, end * i / 3, end * (i + 1) / 3)
            o_to_rhs(ra0, 0, pin, end, T.get('I', 0.88))

        @pl.when(jnp.logical_not(small))
        def _():
            lax.fori_loop(0, H * NQ, attn_guarded, 0)
            lax.fori_loop(0, 3, lambda i, c: (prep_square(i, _no_pin, 0.0, 1.0), c)[1], 0)
            o_to_rhs(ra0, 0, _no_pin, 0.0, 1.0)

        lax.fori_loop(0, NB // 2, mix1_iter, 0)

        @pl.when(l == 1)
        def _():
            for b in range(NB):
                out_copy(b).wait()

        lax.fori_loop(0, NB // 2, mix2_iter, 0)
        return carry

    lax.fori_loop(0, 2, layer, 0)
    for b in range(NB):
        out_copy(b).wait()


@jax.jit
def pallas_interleave_layers__mha_block__mixer_s_mlp__prompt_kernel(
        A_x, A_wqkv, A_wo, B_x, B_w1, B_w2, B_w3, B_w4):
    del B_x
    vmem = pltpu.VMEM
    hbm = pl.BlockSpec(memory_space=pltpu.HBM)
    out = pl.pallas_call(
        _kernel,
        out_shape=jax.ShapeDtypeStruct((D, S), A_x.dtype),
        in_specs=[hbm] * 7,
        out_specs=hbm,
        scratch_shapes=[pltpu.SemaphoreType.DMA((NB + 10,))] + [vmem(*v) for v in SCRATCH.values()],
        compiler_params=pltpu.CompilerParams(vmem_limit_bytes=110 * 2 ** 20),
    )(A_x.reshape(S, D).T, A_wqkv, A_wo, B_w1, B_w2, B_w3, B_w4.T)
    return out.T.reshape(1, S, D)
```

```python
import math

import jax
import jax.numpy as jnp
from jax import lax
from jax.experimental import pallas as pl
from jax.experimental.pallas import tpu as pltpu

S = 2048
D = 448
H = 16
DH = D // H
F = 1792
DHF = D // 2
DHP = 256
FHF = F // 2
DQ = D // 4
NT = 256
TB = 2 * NT
NB = S // TB
NU = F // 256
QB = 512
NQ = S // QB
KC = 128
NC = S // KC
HG = 4
GW = HG * DH
C4 = D // 4
NV = 224
SCORE_BOUND = 90.0
VALUE_BOUND = 2.0 ** 20
EPS = 1e-5
QSCALE = (DH ** -0.5) * math.log2(math.e)

f32 = jnp.float32
bf16 = jnp.bfloat16
u32 = jnp.uint32


def _pack(x):
    return pltpu.bitcast(x.astype(bf16), u32)


def _unpack(x):
    return pltpu.bitcast(x, bf16)


def _rowsum8(x):
    return jnp.sum(x.reshape(x.shape[0] // 8, 8, x.shape[1]), axis=0)


def _colsum(x8):
    return jnp.sum(x8, axis=0, keepdims=True)


def _gelu2(x):
    c = math.sqrt(2.0 / math.pi)
    return x + x * jnp.tanh(x * (c + (c * 0.044715) * (x * x)))


def _dot(a, b):
    return jnp.dot(a, b, preferred_element_type=f32)


def _split(blocks):
    n = len(blocks) // 2
    return ([r[:n] for r in blocks[:n]], [r[n:] for r in blocks[:n]],
            [r[:n] for r in blocks[n:]], [r[n:] for r in blocks[n:]])


def _add(x, y):
    return [[a + b for a, b in zip(r, s)] for r, s in zip(x, y)]


def _sub(x, y):
    return [[a - b for a, b in zip(r, s)] for r, s in zip(x, y)]


def _lhs_terms(blocks):
    if len(blocks) == 1:
        return [blocks[0][0]]
    a11, a12, a21, a22 = _split(blocks)
    terms = (_add(a11, a22), _add(a21, a22), a11, a22, _add(a11, a12), _sub(a21, a11), _sub(a12, a22))
    return [t for x in terms for t in _lhs_terms(x)]


def _rhs_terms(blocks):
    if len(blocks) == 1:
        return [blocks[0][0]]
    b11, b12, b21, b22 = _split(blocks)
    terms = (_add(b11, b22), b11, _sub(b12, b22), _sub(b21, b11), b22, _add(b11, b12), _add(b21, b22))
    return [t for x in terms for t in _rhs_terms(x)]


def _strassen(n, prod, issued, base=0):
    if n == 1:
        issued.append(prod(base))
        return [[issued[-1]]]
    stride = 7 ** (n.bit_length() - 2)

    def m(i):
        return _strassen(n // 2, prod, issued, base + i * stride)

    m1 = m(0)
    m2 = m(1)
    c22 = _sub(m1, m2)
    m4 = m(3)
    c21 = _add(m2, m4)
    c11 = _add(m1, m4)
    m3 = m(2)
    c22 = _add(c22, m3)
    m5 = m(4)
    c12 = _add(m3, m5)
    c11 = _sub(c11, m5)
    c22 = _add(c22, m(5))
    c11 = _add(c11, m(6))
    return [a + b for a, b in zip(c11, c12)] + [a + b for a, b in zip(c21, c22)]


def _join(blocks):
    return jnp.concatenate([jnp.concatenate(r, axis=1) for r in blocks], axis=0)


def _in_ready_order(x, chunks):
    half_r, half_c, lo = x.shape[0] // 2, x.shape[1] // 2, 0
    n = x.shape[0] // sum(chunks)
    for size in chunks:
        for i, j in ((1, 0), (0, 1), (1, 1), (0, 0)):
            for q in range(n // 2):
                r0 = i * half_r + q * sum(chunks) + lo
                yield slice(r0, r0 + size), slice(j * half_c, (j + 1) * half_c)
        lo += size


class _Pins:
    def __init__(self, zero, products, per_product):
        self.keep = lax.broadcasted_iota(jnp.int32, (8, 128), 0) >= zero
        self.points = [m[r:r + 8, 0:128] for m in products
                       for r in range(0, m.shape[0], max(m.shape[0] // per_product // 8, 1) * 8)[:per_product]]

    def at(self, pos):
        return self.points[min(int(pos * len(self.points)), len(self.points) - 1)]

    def __call__(self, v, pos):
        point = self.at(pos)
        if v.dtype != f32:
            point = pltpu.bitcast(point, v.dtype)
        v = jnp.broadcast_to(v, (8, v.shape[1]))
        parts = [v[:, c:c + 128] for c in range(0, v.shape[1], 128)]
        return jnp.concatenate([jnp.where(self.keep, p, point) if p.shape[1] == 128 else p
                                for p in parts], axis=1)


def _no_pin(v, pos):
    return jnp.broadcast_to(v, (8, v.shape[1]))


def _rows(v8, n):
    return jnp.tile(v8, (n // 8, 1))


SCRATCH = dict(
    x_in=((D, S), bf16), wqkv_in=((D, 3 * D), bf16), wsq_in=((3, D, D), bf16),
    w3_in=((D, F), bf16), w4_in=((D, F), bf16),
    wqkv_s=((4, DQ // 2, 49 * 128), u32), wsq_s=((3, DHF // 2, 7 * DHP), u32),
    w3_s=((NU, 32, 49 * 128), u32), w4_s=((49, DQ // 2, 512), u32), w4_t=((8, DHF // 2, FHF), u32),
    xa=((NB // 2, D, TB), f32), xb=((NB // 2, D, TB), f32),
    ya=((NB // 2, D, TB), f32), yb=((NB // 2, D, TB), f32),
    qa=((64, 49 * 128), u32), qb=((64, 49 * 128), u32),
    ra0=((DHP // 2, 7 * NT), u32), rb0=((DHP // 2, 7 * NT), u32), ra1=((DHP // 2, 7 * NT), u32),
    rb1=((DHP // 2, 7 * NT), u32), rg=((DHP // 2, 7 * NT), u32),
    ta=((7, FHF // 2, NT), u32), tf=((F + 32, TB), f32), tb=((192, 49 * 128), u32), sb=((64, 7 * NT), u32),
    qt=((D // 2, S), u32), qf=((H, 32, S), f32), kk=((H // HG, S // 4, 256), u32),
    kb=((32, NV, 128), f32), kf=((2 * H, 32, 256), f32), vt=((H, 16, S), u32), ot=((D, S), f32),
    pbuf=((NQ, S // 2, QB), u32), sbuf=((S, QB), f32),
    hbuf=((D, S + 256), f32), obuf=((D, S), bf16))


def _kernel(x_hbm, wqkv_hbm, wo_hbm, w1_hbm, w2_hbm, w3_hbm, w4_hbm, o_hbm, sems, *scratch):
    named = dict(zip(SCRATCH, scratch))
    (x_in, wqkv_in, wsq_in, w3_in, w4_in, wqkv_s, wsq_s, w3_s, w4_s, w4_t, xa, xb, ya, yb,
     qa, qb, ra0, rb0, ra1, rb1, rg, ta, tf, tb, sb,
     qt, qf, kk, kb, kf, vt, ot, pbuf, sbuf, hbuf, obuf) = [named[n] for n in SCRATCH]

    def x_copy(b):
        cols = pl.ds(b * TB, TB)
        return pltpu.make_async_copy(x_hbm.at[:, cols], x_in.at[:, cols], sems.at[b])

    def out_copy(b):
        cols = pl.ds(pl.multiple_of(b * TB, TB), TB)
        return pltpu.make_async_copy(obuf.at[:, cols], o_hbm.at[:, cols], sems.at[b])

    w_copies = [pltpu.make_async_copy(src, dst, sems.at[NB + 1 + i]) for i, (src, dst) in enumerate((
        (wo_hbm, wsq_in.at[0]), (w1_hbm, wsq_in.at[1]), (w2_hbm, wsq_in.at[2]), (w3_hbm, w3_in), (w4_hbm, w4_in)))]
    qkv_copies = [pltpu.make_async_copy(wqkv_hbm.at[pl.ds(j * DQ, DQ)], wqkv_in.at[pl.ds(j * DQ, DQ)],
                                        sems.at[NB + 6 + j]) for j in range(4)]
    x_copy(0).start()
    for c in qkv_copies:
        c.start()
    for b in range(1, NB):
        x_copy(b).start()

    hbuf[:, 0:128] = jnp.zeros((D, 128), f32)
    hbuf[:, S + 128:S + 256] = jnp.zeros((D, 128), f32)
    for r in (ra0, rb0, ra1, rb1, rg):
        r[DHF // 2:, :] = jnp.zeros(((DHP - DHF) // 2, 7 * NT), u32)
    for r in (qa, qb):
        r[DQ // 2:, :] = jnp.zeros((64 - DQ // 2, 49 * 128), u32)

    def tile(i):
        return slice(i * 128, (i + 1) * 128)

    def tokens(b):
        return pl.ds(pl.multiple_of(b * TB, TB), TB)

    def prep_weight(load, dst, n, rows_out, pin, lo, hi):
        parts = []
        mid = lo + (hi - lo) * 0.4
        for j in range(n):
            w = load(slice(j * D // n, (j + 1) * D // n)).astype(f32)
            m = w.shape[1]
            w = jnp.concatenate([pin(w[0:8], lo + (mid - lo) * j / n), w[8:], jnp.zeros(((512 - D) // n, m), f32)], axis=0)
            parts.append(w.T)
        for j in range(m // (n * rows_out)):
            for r in range(0, rows_out, 16):
                grid = [[p[(n * j + i) * rows_out + r:(n * j + i) * rows_out + r + 16] for p in parts] for i in range(n)]
                if pin is not _no_pin:
                    pos = mid + (hi - mid) * r / rows_out
                    grid = [[jnp.concatenate([pin(x[0:8], pos), pin(x[8:16], pos)], axis=0) for x in g] for g in grid]
                for i, t in enumerate(_lhs_terms(grid)):
                    dst(j)[r // 2:r // 2 + 8, i * 512 // n:(i + 1) * 512 // n] = _pack(t)
        return parts

    def rhs_terms(grid, pin, pos):
        if len(grid) == 2:
            return _rhs_terms(grid)
        b11, b12, b21, b22 = _split(grid)

        def late(blocks, j):
            return [[jnp.concatenate([pin(x[0:8], pos((j + 1) / 8)), pin(x[8:16], pos((j + 1) / 8))], axis=0)
                     for x in r] for r in blocks]
        b11, b22, b12, b21 = late(b11, 0), late(b22, 1), late(b12, 3), late(b21, 5)
        outer = (_add(b11, b22), b11, _sub(b12, b22), _sub(b21, b11), b22, _add(b11, b12), _add(b21, b22))
        return [t for x in outer for t in _rhs_terms(x)]

    def put_rhs(dst, piece, pin=None, pos=None):
        n = 256 // dst.shape[0]
        for k in range(D // n // 16):
            rows = [piece(slice(i * D // n + k * 16, i * D // n + (k + 1) * 16), k) for i in range(n)]
            grid = [[x[:, c:c + TB // n] for c in range(0, TB, TB // n)] for x in rows]
            for i, t in enumerate(rhs_terms(grid, pin, lambda f: pos(k + f))):
                dst[k * 8:(k + 1) * 8, i * TB // n:(i + 1) * TB // n] = _pack(t)

    def matmul(w, base, rhs, z, chunks=None):
        n = 256 // rhs.shape[0]
        rows = pl.ds(pl.multiple_of(z * 8, 8), rhs.shape[0])
        issued, grids, lo = [], [], 0
        for size in chunks or (2 * w.shape[1],):
            part = slice(lo // 2, (lo + size) // 2)
            grids.append(_strassen(n, lambda i: _dot(_unpack(w[base, part, i * 512 // n:(i + 1) * 512 // n]),
                                                     _unpack(rhs[rows, i * TB // n:(i + 1) * TB // n])), issued))
            lo += size
        return _join([r for i in range(n) for r in (g[i] for g in grids)]), issued

    def update(ref, it, a, chunks, new):
        sums = {}
        for rows, cols in _in_ready_order(a, chunks):
            x = new(rows, cols, a[rows, cols])
            ref.at[it][rows, cols] = x
            sums[cols.start] = _rowsum8(x) + sums[cols.start] if cols.start in sums else _rowsum8(x)
        return jnp.concatenate([sums[0], sums[NT]], axis=1)

    def ln_stats(load, s8, pin, lo, hi, n=14):
        mean = _colsum(s8) * (1.0 / D)
        step = D // n
        v8 = None
        for k in range(n):
            xc = load(slice(k * step, (k + 1) * step)) - _rows(pin(mean, lo + (hi - lo) * k / n), step)
            v8 = _rowsum8(xc * xc) if v8 is None else v8 + _rowsum8(xc * xc)
        var = _colsum(v8) * (1.0 / D)
        return mean, lax.rsqrt(var + EPS), var

    def ln_to_rhs(dst, load1, load2, s8, pin, lo, hi, n=7):
        mid = lo + (hi - lo) * 0.33
        mean, rstd, _ = ln_stats(load1, s8, pin, lo, mid)
        means = [pin(mean, mid + (hi - mid) * k / n) for k in range(n)]
        put_rhs(dst, lambda rows, k: (load2(rows) - _rows(means[k], 16)) * rstd,
                pin, lambda k: mid + (hi - mid) * k / n)

    def first_ln(dst, xs, it, z1, z2, pin, lo, hi, n=4):
        mid = lo + (hi - lo) * 0.15
        step = D // n
        s8 = None
        for k in range(n):
            x = xs[it + z2, k * step:(k + 1) * step, :]
            x = jnp.concatenate([pin(x[0:8], lo + (mid - lo) * k / n), x[8:]], axis=0)
            s8 = _rowsum8(x) if s8 is None else s8 + _rowsum8(x)
        ln_to_rhs(dst, lambda rows: xs[it + z1, rows, :], lambda rows: xs[it + z2, rows, :], s8, pin, mid, hi)

    def o_to_rhs(dst, b, pin, lo, hi, n=14):
        ones = [pin(jnp.ones((8, TB), f32), lo + (hi - lo) * k / n) for k in range(n)]
        put_rhs(dst, lambda rows, k: ot[rows, tokens(b)] * _rows(ones[k], 16))

    def shifted_to_rhs(dst, b, pin, lo, hi, valid=1):
        n = 14
        keeps = [pin(jnp.full((8, 128), valid, jnp.int32), lo + (hi - lo) * k / n) for k in range(n)]

        def piece(rows, k):
            sh = (1, -1, 2, -2)[rows.start // C4]
            w = hbuf[rows, pl.ds(pl.multiple_of(b * TB, TB), TB + 256)]
            g = w[:, 128 - sh:128 - sh + TB]
            return jnp.where(jnp.tile(keeps[k], (g.shape[0] // 8, TB // 128)) == 1, g, 0.0)
        put_rhs(dst, piece)

    def convert(b):
        x_copy(b).wait()
        (xa, xb)[b % 2][b // 2] = x_in[:, b * TB:(b + 1) * TB].astype(f32)

    def qkv_rows(rows):
        qkv_copies[rows.start // DQ].wait()
        return wqkv_in[rows, :]

    convert(0)
    first_ln(qa, xa, 0, 0, 0, _no_pin, 0.0, 1.0)
    parts = prep_weight(qkv_rows, lambda j: wqkv_s.at[j], 4, DQ, _no_pin, 0.0, 1.0)
    v_max = D * jnp.max(jnp.abs(jnp.concatenate([p[2 * D:] for p in parts], axis=0)))
    for c in w_copies:
        c.start()
    convert(1)
    convert(2)

    def window(x, h):
        r0 = (DH * h) // 8 * 8
        return x[r0:r0 + 32, :]

    def head_rows(x, h):
        w = window(x, h)
        if h % 2:
            row = lax.broadcasted_iota(jnp.int32, (8, x.shape[1]), 0)
            w = jnp.concatenate([jnp.where(row < 4, pltpu.roll(w[24:32], 4, 0), w[0:8]), w[8:32]], axis=0)
        return w

    def lane_tiles_max(x):
        out = x[:, 0:128]
        for c in range(128, x.shape[1], 128):
            out = jnp.maximum(out, x[:, c:c + 128])
        return out

    def max_norm2(x):
        sq = x * x
        out = None
        for h in range(HG):
            n2 = _colsum(_rowsum8(window(sq, h)))
            out = n2 if out is None else jnp.maximum(out, n2)
        return lane_tiles_max(out)

    def project(b, odd, rhs, z, k2):
        def ready(x):
            for rows, cols in _in_ready_order(x, (DQ,)):
                yield rows.start // DQ, x[rows, cols], cols.start

        def at(t0):
            return pl.ds(pl.multiple_of(b * TB + t0, NT), NT)

        k, pk = matmul(wqkv_s, 1, rhs, z)
        for g, x, t0 in ready(k):
            kg = jnp.concatenate([x, jnp.zeros((128 - GW, NT), f32)], axis=0)
            rows = pl.ds(pl.multiple_of((b // 2 * TB + t0) // 2, NT // 2), NT // 2)
            kk.at[g][rows, tile(odd)] = _pack(kg.T)
            k2 = jnp.maximum(k2, max_norm2(x))
            if not odd and t0 == 0:
                for j in range(HG):
                    kf.at[b // 2 * H + g * HG + j][...] = head_rows(x, j)
        v, pv = matmul(wqkv_s, 2, rhs, z)
        row = lax.broadcasted_iota(jnp.int32, (8, NT), 0)
        for g, x, t0 in ready(v):
            for j in range(HG):
                w = window(x, j)
                if j % 2 == 0:
                    w = jnp.concatenate([w[0:24], jnp.where(row < 4, w[24:32], 1.0)], axis=0)
                else:
                    w = jnp.concatenate([jnp.where(row >= 4, w[0:8], 1.0), w[8:32]], axis=0)
                vt.at[g * HG + j][:, at(t0)] = _pack(w)
        q, pq = matmul(wqkv_s, 0, rhs, z)
        for g, x, t0 in ready(q):
            x = x * QSCALE
            qt[g * GW // 2:(g + 1) * GW // 2, at(t0)] = _pack(x)
            for j in range(HG):
                qf.at[g * HG + j][:, at(t0)] = head_rows(x, j)
        return _Pins(z, pk + pv + pq, 1), k2

    def keys(h, lo, n):
        block, row = lo // TB, lo % TB
        return _unpack(kk[h // HG, (block // 2 * TB + row) // 2:(block // 2 * TB + row + n) // 2, tile(block % 2)])

    def spread_keys(h, t, pin, lo, hi):
        n = min(NV - 128 * t, 128)
        for d in range(DH):
            row = pin(kf[h, d:d + 1, tile(t)], lo + (hi - lo) * d / DH)
            kb.at[d][128 * t:128 * t + n, :] = _rows(row[:, 0:n], 128).T

    def prep_square(i, pin, lo, hi):
        prep_weight(lambda rows: wsq_in[i, rows, :], lambda j: wsq_s.at[i], 2, DHF, pin, lo, hi)

    def prep_up(u, pin, lo, hi):
        cols = pl.ds(u * 256 if isinstance(u, int) else pl.multiple_of(u * 256, 256), 256)
        prep_weight(lambda rows: w3_in[rows, cols], lambda _: w3_s.at[u], 4, 64, pin, lo, hi)

    def prep_down2(p, _):
        low = lax.broadcasted_iota(jnp.int32, (16, 128), 1) < 64

        def piece(r, _):
            grid = []
            for i in range(4):
                rows = pl.ds(pl.multiple_of(i * DQ + r * 16, 16), 16)
                w = w4_in[rows, pl.ds(pl.multiple_of(p * 512, 512), 512)].astype(f32)
                t = [w[:, tile(c)] for c in range(4)]
                grid.append([jnp.where(low, t[0], pltpu.roll(t[2], 64, 1)), jnp.where(low, pltpu.roll(t[0], 64, 1), t[2]),
                             jnp.where(low, t[1], pltpu.roll(t[3], 64, 1)), jnp.where(low, pltpu.roll(t[1], 64, 1), t[3])])
            for i, term in enumerate(_lhs_terms(grid)):
                w4_s.at[i][pl.ds(pl.multiple_of(r * 8, 8), 8), pl.ds(pl.multiple_of(p * 128, 128), 128)] = _pack(term)
            return 0

        return lax.fori_loop(0, DQ // 16, piece, 0, unroll=True)

    def prep_down1(u, _):
        cols = pl.ds(pl.multiple_of(u * 256, 256), 256)
        for r in range(0, DHF, 32):
            top = w4_in[r:r + 32, cols].astype(f32)
            bot = w4_in[DHF + r:DHF + r + 32, cols].astype(f32)
            for i, t in enumerate(_lhs_terms([[top[:, :128], top[:, 128:]], [bot[:, :128], bot[:, 128:]]])):
                w4_t.at[i][r // 2:r // 2 + 16, pl.ds(pl.multiple_of(u * 128, 128), 128)] = _pack(t)
        return 0

    def qkv_iter(l, it, k2):
        @pl.when(jnp.logical_and(l == 0, it == 1))
        def _():
            convert(3)

        z1, z2 = lax.shift_right_logical(it, 8), lax.shift_right_logical(it, 9)
        nxt = jnp.minimum(it + 1, NB // 2 - 1)
        pin, k2 = project(2 * it, 0, qa, z1, k2)
        first_ln(qb, xb, it, z1, z2, pin, 0.064, 0.866)
        pin, k2 = project(2 * it + 1, 1, qb, z1, k2)
        first_ln(qa, xa, nxt, z1, z2, pin, 0.02, 0.849)
        return k2

    def finish_head(acc, hp, qbp):
        odd = hp % 2
        l = jnp.where(odd == 1, acc[0:1, :], acc[28:29, :])
        o = acc * (1.0 / l)
        r0 = pl.multiple_of((DH * hp) // 8 * 8, 8)
        cols = pl.ds(qbp * QB if isinstance(qbp, int) else pl.multiple_of(qbp * QB, QB), QB)
        row = lax.broadcasted_iota(jnp.int32, (8, QB), 0)
        ot[pl.ds(r0, 8), cols] = jnp.where(row >= 4 * odd, o[0:8], ot[pl.ds(r0, 8), cols])
        ot[pl.ds(r0 + 8, 24), cols] = o[8:32]

    def masked_q(h, cols):
        g0 = (h // HG) * (GW // 2)
        qg = qt[pl.ds(g0 if isinstance(g0, int) else pl.multiple_of(g0, 8), GW // 2), cols]
        row = lax.broadcasted_iota(jnp.int32, (GW // 2, QB), 0)
        lo = (h % HG) * (DH // 2)
        qm = jnp.where((row >= lo) & (row < lo + DH // 2), qg, jnp.zeros_like(qg))
        return _unpack(jnp.concatenate([qm, jnp.zeros(((128 - GW) // 2, QB), u32)], axis=0))

    def attn_head(h, last=False):
        hp = h - 1
        products = []

        def weighted(u, c):
            d = _dot(_unpack(vt[hp, :, c * KC:(c + 1) * KC]), _unpack(pbuf[u, c * KC // 2:(c + 1) * KC // 2, :]))
            products.append(d)
            return d

        early = pl.cdiv(NV, KC)
        accs = [sum(weighted(u, c) for c in range(1, early)) + weighted(u, 0) for u in range(NQ)]
        for u in range(NQ):
            qm = None if last else masked_q(h, slice(u * QB, (u + 1) * QB))
            acc = accs[u]
            for c in range(NC):
                lo, hi = max(c * KC, NV), (c + 1) * KC
                first = u == NQ - 1 and c == NC - 1
                if first:
                    acc = acc + weighted(u, c)
                if hi > lo and not last:
                    st = _dot(keys(h, lo, hi - lo), qm)
                    products += [st[r:r + 32] for r in range(0, hi - lo, 32)]
                if c >= early and not first:
                    acc = acc + weighted(u, c)
                if hi > lo and not last:
                    pbuf.at[u][lo // 2:hi // 2, :] = _pack(jnp.exp2(st))
            finish_head(acc, hp, u)
        pin = _Pins(lax.shift_right_logical(h, 10), products, 4)
        if last:
            return pin
        units = [(u, r0, t0) for r0 in range(0, NV, 16) for u in range(NQ) for t0 in (0, 2)]

        def pos(n, d):
            return (n + d / DH) / len(units) * 0.993 - 0.008

        spread_keys(h, 1, pin, 0.057, 0.267)
        for n, (u, r0, t0) in enumerate(units):
            acc = {}
            for d in range(DH):
                ks = [kb[d, r:r + 8, :] for r in (r0, r0 + 8)]
                if d % 4 == 0 and pos(n, d) >= 0:
                    ks = [pin(k, pos(n, d)) for k in ks]
                for t in (t0, t0 + 1):
                    q = jnp.broadcast_to(qf[h, d:d + 1, tile(u * (QB // 128) + t)], (8, 128))
                    for r in range(2):
                        acc[r, t] = ks[r] * q if d == 0 else acc[r, t] + ks[r] * q
            for t in (t0, t0 + 1):
                st = jnp.concatenate([acc[0, t], acc[1, t]], axis=0)
                pbuf.at[u][r0 // 2:r0 // 2 + 8, t * 128:(t + 1) * 128] = _pack(jnp.exp2(st))
        done = {r0: n + 1 for n, (u, r0, t0) in enumerate(units)}
        nxt = jnp.minimum(h + 1, H - 1)
        spread_keys(nxt, 0, pin, pos(done[128 - 16], 0), 0.882)
        return pin

    def attn_first(j, q2, k2):
        products = []
        for u in (2 * j, 2 * j + 1):
            qm = masked_q(0, pl.ds(pl.multiple_of(u * QB, QB), QB))
            for c in range(NC):
                st = _dot(keys(0, c * KC, KC), qm)
                pbuf.at[u][c * KC // 2:(c + 1) * KC // 2, :] = _pack(jnp.exp2(st))
                products.append(st)
        pin = _Pins(lax.shift_right_logical(j, 10), products, 8)
        end = 0.688
        for i in range(3):
            prep_up(3 * j + i, pin, end * i / 3, end * (i + 1) / 3)
        for r in (0, 8):
            rows = kf[1, pl.ds(pl.multiple_of(16 * j + r, 8), 8), tile(0)]
            for d in range(8):
                pos = 0.72 + 0.15 * (r + d) / 16
                kb.at[16 * j + r + d][0:128, :] = _rows(pin(rows[d:d + 1], pos), 128).T
        for h in range(H):
            x = qf[h, :, pl.ds(pl.multiple_of(j * (S // 2), S // 2), S // 2)]
            x = jnp.concatenate([pin(x[0:8], 0.875 * h / H), x[8:]], axis=0)
            q2 = jnp.maximum(q2, lane_tiles_max(_colsum(_rowsum8(x * x))))
        small = jnp.logical_and(jnp.max(q2) * jnp.max(k2) <= SCORE_BOUND ** 2, v_max <= VALUE_BOUND)
        return q2, small.astype(jnp.int32)

    def attn_guarded(i, _):
        h, cols = i // NQ, pl.ds(pl.multiple_of((i % NQ) * QB, QB), QB)
        qm = masked_q(h, cols)

        def scores(c, m):
            rows = pl.ds(pl.multiple_of(c * (KC // 2), KC // 2), KC // 2)
            first = c // (TB // KC) * 2 * TB + c % (TB // KC) * KC
            for odd in range(2):
                st = _dot(_unpack(kk[h // HG, rows, tile(odd)]), qm)
                sbuf[pl.ds(pl.multiple_of(first + odd * TB, KC), KC), :] = st
                m = jnp.maximum(m, jnp.max(st, axis=0, keepdims=True))
            return m

        m = lax.fori_loop(0, NC // 2, scores, jnp.full((1, QB), -jnp.inf, f32))

        def weighted(c, acc):
            rows = pl.ds(pl.multiple_of(c * KC, KC), KC)
            return acc + _dot(_unpack(vt[h, :, rows]), jnp.exp2(sbuf[rows, :] - m).astype(bf16))

        finish_head(lax.fori_loop(0, NC, weighted, jnp.zeros((32, QB), f32)), h, i % NQ)
        return 0

    def mix1_iter(it, _):
        z1, z2 = lax.shift_right_logical(it, 8), lax.shift_right_logical(it, 9)
        nxt = jnp.minimum(it + 1, NB // 2 - 1)

        def add_out_proj(xs, rhs):
            chunks = (112, 112)
            a, products = matmul(wsq_s, 0, rhs, z1, chunks)
            return update(xs, it, a, chunks, lambda r, c, v: xs[it, r, c] + v), _Pins(z1, products, 4)

        def two_norms(dst, xs, ys, s8, pin, n=14):
            mean, rstd, var = ln_stats(lambda rows: xs[it + z1, rows, :], s8, pin, 0.0, 0.195)
            rstd2 = lax.rsqrt(var * rstd * rstd + EPS)
            means = [pin(mean, 0.236 + (0.825 - 0.236) * k / n) for k in range(n)]

            def piece(rows, k):
                y = (xs[it + z2, rows, :] - _rows(means[k], rows.stop - rows.start)) * rstd
                ys.at[it][rows, :] = y
                return y * rstd2
            put_rhs(dst, piece)

        def hidden(b, rhs):
            chunks = (112, 112)
            h, products = matmul(wsq_s, 1, rhs, z1, chunks)
            for rows, cols in _in_ready_order(h, chunks):
                hbuf[rows, pl.ds(pl.multiple_of(b * TB + 128 + cols.start, 128), NT)] = _gelu2(h[rows, cols])
            return _Pins(z1, products, 4)

        suma, pin = add_out_proj(xa, ra0)
        o_to_rhs(rb0, 2 * it + 1, pin, 0.0, 0.441)
        shifted_to_rhs(rg, 0, pin, 0.441, 0.901, valid=it)
        sumb, pin = add_out_proj(xb, rb0)
        two_norms(ra1, xa, ya, suma, pin)
        pin = hidden(2 * it, ra1)
        two_norms(rb1, xb, yb, sumb, pin)
        pin = hidden(2 * it + 1, rb1)
        o_to_rhs(ra0, 2 * nxt, pin, 0.03, 0.627)
        return 0

    def mix2_iter(it, _):
        z1, z2 = lax.shift_right_logical(it, 8), lax.shift_right_logical(it, 9)
        nxt = jnp.minimum(it + 1, NB // 2 - 1)

        def add_mixer(ys, rhs):
            chunks = (112, 112)
            a, products = matmul(wsq_s, 2, rhs, z1, chunks)
            return update(ys, it, a, chunks, lambda r, c, v: ys[it, r, c] + 0.5 * v), _Pins(z1, products, 4)

        def norm(dst, ys, s8, pin, end):
            ln_to_rhs(dst, lambda rows: ys[it + z1, rows, :], lambda rows: ys[it + z2, rows, :],
                      s8, pin, 0.0, end)

        def up(rhs, put):
            pins = []
            for u in range(NU):
                t, issued = matmul(w3_s, u, rhs, z1, (32, 32))
                put(u, _gelu2(t))
                pins += issued
            return _Pins(z1, pins, 1)

        def halves(t):
            return [[t[:128, :NT], t[:128, NT:]], [t[128:, :NT], t[128:, NT:]]]

        def put_a(u, t):
            for i, term in enumerate(_rhs_terms(halves(t))):
                ta.at[i][u * 64:(u + 1) * 64, :] = _pack(term)

        def put_b(u, t):
            tf[u * 256:(u + 1) * 256, :] = t

        def down_a():
            products, grids, lo = [], [], 0
            for size in (32,) * 7:
                part = slice(lo // 2, (lo + size) // 2)
                grids.append(_strassen(2, lambda i: _dot(_unpack(w4_t[i, part, :]), _unpack(ta[i + z1])), products))
                lo += size
            return _join([g[i] for i in range(2) for g in grids]), _Pins(z1, products, 8)

        def split_b(pin, end):
            view = tf.at[pl.ds(pl.multiple_of(z1 * 8, 8), F)]

            def hidden(lo, n):
                return view[lo:lo + n, :]

            for r in range(0, 128, 16):
                top, bot = hidden((NU - 1) * 256 + r, 16), hidden((NU - 1) * 256 + 128 + r, 16)
                top, bot = [jnp.concatenate([pin(x[j:j + 8], end * (r / 128) / (4 * NU - 3)) for j in (0, 8)], axis=0)
                            for x in (top, bot)]
                for i, term in enumerate(_rhs_terms([[top[:, :NT], top[:, NT:]], [bot[:, :NT], bot[:, NT:]]])):
                    sb[r // 2:r // 2 + 8, i * NT:(i + 1) * NT] = _pack(term)
            for k in range(4 * (NU - 1)):
                rows = [hidden(k // 4 * 256 + i * 64 + k % 4 * 16, 16) for i in range(4)]
                grid = [[x[:, tile(c)] for c in range(4)] for x in rows]
                for i, term in enumerate(rhs_terms(grid, pin, lambda f: end * (k + 1 + f) / (4 * NU - 3))):
                    tb[k * 8:(k + 1) * 8, tile(i)] = _pack(term)

        def down_b():
            tail = _join(_strassen(2, lambda i: _dot(
                _unpack(w4_t[i, :, tile(NU - 1)]),
                _unpack(sb[pl.ds(pl.multiple_of(z1 * 8, 8), 64), i * NT:(i + 1) * NT])), []))
            products, grids, lo = [], [], 0
            for size in (64, 48):
                part = slice(lo // 2, (lo + size) // 2)
                grids.append(_strassen(4, lambda i: _dot(_unpack(w4_s[i, part, 0:384]),
                                                         _unpack(tb[pl.ds(pl.multiple_of(z1 * 8, 8), 192), tile(i)])), products))
                lo += size
            return _join([g[i] for i in range(4) for g in grids]) + tail, _Pins(z1, products, 1)

        def down(b, xs, ys, a, chunks):
            def new(rows, cols, v):
                x = xs[it, rows, cols] + (ys[it + z1, rows, cols] + 0.5 * v)
                obuf[rows, pl.ds(pl.multiple_of(b * TB + cols.start, NT), NT)] = x.astype(bf16)
                return x
            update(xs, it, a, chunks, new)

        suma, pin = add_mixer(ya, rg)
        shifted_to_rhs(rb0, 2 * it + 1, pin, 0.0, 0.832)
        sumb, pin = add_mixer(yb, rb0)
        norm(qa, ya, suma, pin, 0.864)
        pin = up(qa, put_a)
        norm(qb, yb, sumb, pin, 0.939)
        up(qb, put_b)
        a, pin = down_a()
        down(2 * it, xa, ya, a, (32,) * 7)
        split_b(pin, 0.74)
        a, pin = down_b()
        out_copy(2 * it).start()
        down(2 * it + 1, xb, yb, a, (64, 48))
        shifted_to_rhs(rg, 2 * nxt, pin, 0.0, 0.206)
        first_ln(qa, xa, 0, z1, z2, pin, 0.206, 0.894)
        out_copy(2 * it + 1).start()
        return 0

    def layer(l, carry):
        zero = jnp.zeros((1, 128), f32)
        k2 = lax.fori_loop(0, NB // 2, lambda it, c: qkv_iter(l, it, c), zero)

        @pl.when(l == 0)
        def _():
            for c in w_copies:
                c.wait()
            lax.fori_loop(0, NU, prep_down1, 0)
            lax.fori_loop(0, NU // 2, prep_down2, 0)
            prep_up(NU - 1, _no_pin, 0.0, 1.0)
            prep_square(2, _no_pin, 0.0, 1.0)

        _, small = lax.fori_loop(0, NQ // 2, lambda j, c: attn_first(j, c[0], k2), (zero, jnp.int32(0)))
        small = small == 1

        @pl.when(small)
        def _():
            lax.fori_loop(1, H, lambda h, c: (attn_head(h), c)[1], 0)
            pin = attn_head(l * 0 + H, last=True)
            end = 0.5
            for i in range(2):
                prep_square(i, pin, end * i / 2, end * (i + 1) / 2)
            o_to_rhs(ra0, 0, pin, end, 0.75)

        @pl.when(jnp.logical_not(small))
        def _():
            lax.fori_loop(0, H * NQ, attn_guarded, 0)
            lax.fori_loop(0, 2, lambda i, c: (prep_square(i, _no_pin, 0.0, 1.0), c)[1], 0)
            o_to_rhs(ra0, 0, _no_pin, 0.0, 1.0)

        lax.fori_loop(0, NB // 2, mix1_iter, 0)

        @pl.when(l == 1)
        def _():
            for b in range(NB):
                out_copy(b).wait()

        lax.fori_loop(0, NB // 2, mix2_iter, 0)
        return carry

    lax.fori_loop(0, 2, layer, 0)
    for b in range(NB):
        out_copy(b).wait()


@jax.jit
def pallas_interleave_layers__mha_block__mixer_s_mlp__prompt_kernel(
        A_x, A_wqkv, A_wo, B_x, B_w1, B_w2, B_w3, B_w4):
    del B_x
    vmem = pltpu.VMEM
    hbm = pl.BlockSpec(memory_space=pltpu.HBM)
    out = pl.pallas_call(
        _kernel,
        out_shape=jax.ShapeDtypeStruct((D, S), A_x.dtype),
        in_specs=[hbm] * 7,
        out_specs=hbm,
        scratch_shapes=[pltpu.SemaphoreType.DMA((NB + 10,))] + [vmem(*v) for v in SCRATCH.values()],
        compiler_params=pltpu.CompilerParams(vmem_limit_bytes=110 * 2 ** 20),
    )(A_x.reshape(S, D).T, A_wqkv, A_wo, B_w1, B_w2, B_w3, B_w4.T)
    return out.T.reshape(1, S, D)
```
